```python
import os as _os
_os.environ.setdefault("JAX_PLATFORMS", "cpu")
import jax
import jax.numpy as jnp

def _softmax(x, axis=-1):
    return jax.nn.softmax(x, axis=axis)
def _gelu(x):
    return jax.nn.gelu(x, approximate=True)
def _silu(x):
    return jax.nn.silu(x)
def _sigmoid(x):
    return jax.nn.sigmoid(x)
def _layernorm(x, axis=-1, eps=1e-5):
    m = jnp.mean(x, axis=axis, keepdims=True)
    v = jnp.var(x, axis=axis, keepdims=True)
    return (x - m) / jnp.sqrt(v + eps)
def _scatter_add(tgt, idx, src, axis=0):
    return tgt.at[idx].add(src)
def _segment_sum(src, seg, n):
    return jax.ops.segment_sum(src, seg, n)
class _Rng:
    def __init__(self, key):
        self._k = key
    def _next(self):
        self._k, sub = jax.random.split(self._k)
        return sub
    def normal(self, shape):
        return jax.random.normal(self._next(), shape, dtype=jnp.bfloat16)
    def randint(self, lo, hi, shape):
        return jax.random.randint(self._next(), shape, lo, hi, dtype=jnp.int32)
    def uniform(self, shape, lo=0.0, hi=1.0):
        return jax.random.uniform(self._next(), shape, jnp.bfloat16, lo, hi)
    def permutation(self, n):
        return jax.random.permutation(self._next(), n)


kernel_name = 'interleave_layers__sliding_block_cached__mixer_channel_mlp__decode'

def setup_inputs():
    _rng = _Rng(jax.random.key(int.from_bytes(__import__("os").urandom(4), "little")))
    _w = (lambda a: (lambda t: t.astype(jnp.bfloat16) if jnp.issubdtype(t.dtype, jnp.floating) else t)(jnp.asarray(a)))
    def _A_setup():
        B, Sq, D = 8, 1, 640
        Hq, Hkv, Sk, Dh = 32, 32, 4096, 128
        assert Hq % Hkv == 0, (Hq, Hkv)
        return {
            "x": _w((lambda *s: _rng.normal(s) * 0.05)(B, Sq, D)),
            "k_cache": _w((lambda *s: _rng.normal(s) * 1.6)(B, Hkv, Sk, Dh)),
            "v_cache": _w((lambda *s: _rng.normal(s) * 0.8)(B, Hkv, Sk, Dh)),
            "wq": _w((lambda *s: _rng.normal(s) * 1.6)(D, Hq * Dh) * (D ** -0.5)),
            "wo": _w((lambda *s: _rng.normal(s) * 0.8)(Hq * Dh, D) * ((Hq * Dh) ** -0.5)),
        }
    _A_in = _A_setup()

    def _B_setup():
        B, S, D, F = 8, 1, 640, 1728
        return {
            "x": _w((lambda *s: _rng.normal(s) * 0.05)(B, S, D)),
            "w1": _w((lambda *s: _rng.normal(s) * 0.4)(D, F) * (D ** -0.5)),
            "b1": _w((lambda *s: _rng.normal(s) * 0.4)(F)),
            "w2": _w((lambda *s: _rng.normal(s) * 0.4)(F, D) * (F ** -0.5)),
            "b2": _w((lambda *s: _rng.normal(s) * 0.2)(D)),
        }
    _B_in = _B_setup()

    return {
        "A_x": _A_in["x"],
        "A_k_cache": _A_in["k_cache"],
        "A_v_cache": _A_in["v_cache"],
        "A_wq": _A_in["wq"],
        "A_wo": _A_in["wo"],
        "B_x": _B_in["x"],
        "B_w1": _B_in["w1"],
        "B_b1": _B_in["b1"],
        "B_w2": _B_in["w2"],
        "B_b2": _B_in["b2"],
    }

def reference(A_x, A_k_cache, A_v_cache, A_wq, A_wo, B_x, B_w1, B_b1, B_w2, B_b2):
    def _A_ref(x, k_cache, v_cache, wq, wo):
        B, Sq, D = x.shape
        Hq, Dh = 32, 128
        Hkv, Sk = k_cache.shape[1], k_cache.shape[2]
        W = min(4096, max(256, Sk // 4))
        rep = Hq // Hkv
        q = (lambda x, *d: x.transpose(*d))((x @ wq).reshape(B, Sq, Hq, Dh), 0, 2, 1, 3)
        k = jnp.repeat(k_cache[:, :, Sk - W:, :], rep, axis=1)
        v = jnp.repeat(v_cache[:, :, Sk - W:, :], rep, axis=1)
        scores = jnp.einsum("bhqd,bhkd->bhqk", q, k) * (Dh ** -0.5)
        p = _softmax(scores, axis=-1)
        o = jnp.einsum("bhqk,bhkd->bhqd", p, v)
        return (lambda x, *d: x.transpose(*d))(o, 0, 2, 1, 3).reshape(B, Sq, Hq * Dh) @ wo

    def _B_ref(x, w1, b1, w2, b2):
        y = _layernorm(x, axis=-1)
        h = _gelu(jnp.einsum("bsd,df->bsf", y, w1) + b1)
        return jnp.einsum("bsf,fd->bsd", h, w2) + b2

    x = A_x
    x = x + _A_ref(_layernorm(x, axis=-1), A_k_cache, A_v_cache, A_wq, A_wo)
    x = x + _B_ref(_layernorm(x, axis=-1), B_w1, B_b1, B_w2, B_b2)
    x = x + _A_ref(_layernorm(x, axis=-1), A_k_cache, A_v_cache, A_wq, A_wo)
    x = x + _B_ref(_layernorm(x, axis=-1), B_w1, B_b1, B_w2, B_b2)
    return x
```

```python
import functools

import jax
import jax.numpy as jnp
from jax import lax
import jax.experimental.pallas as pl
import jax.experimental.pallas.tpu as pltpu

BF16 = jnp.bfloat16
F32 = jnp.float32
U32 = jnp.uint32

B, D, H, SK, DH, F = 8, 640, 32, 4096, 128, 1728
W = min(4096, max(256, SK // 4))
G = 8
NG = H // G
ND = D // 128
NF = -(-F // 128)
NT = W // 128
ROWS = 8
NCOPY = W // 2 // ROWS
EPS = 1e-5
QSCALE = (DH ** -0.5) * 1.4426950408889634


def _gelu(x):
    c = 0.7978845608028654
    return 0.5 * x * (1.0 + jnp.tanh(c * (x + 0.044715 * (x * x * x))))


def _bf(x):
    return pltpu.bitcast(x, BF16)


def _moments(x):
    m = jnp.mean(x, axis=-1, keepdims=True)
    c = x - m
    return m, jnp.mean(c, axis=-1, keepdims=True), jnp.mean(c * c, axis=-1, keepdims=True)


def _column(r):
    return jnp.concatenate([r] * 16, axis=0).T


def _vpu_dot(load, col, acc):
    part = [None] * len(acc)
    for i in range(16):
        ci = col[i * 8:(i + 1) * 8, :]
        for t in range(len(acc)):
            term = load(i, t) * ci
            part[t] = term if i == 0 else part[t] + term
    return [p if a is None else a + p for a, p in zip(acc, part)]


def _emit(*streams):
    tasks = []
    for stream in streams:
        now = 0
        for fn, arg, start, cost in stream:
            now = max(now, start)
            tasks.append((now, len(tasks), fn, arg))
            now += cost
    for _, _, fn, arg in sorted(tasks, key=lambda t: t[:2]):
        fn(arg)


def _kernel(opts, x_hbm, k_hbm, v_hbm, wq_hbm, wo_hbm, w1_hbm, b1_hbm, w2_hbm, b2_hbm, o_ref,
            kbuf, vbuf, kt, wq_v, wo_v, w1_v, w2_v, wq_p, wo_p, w1_p, w2_p, wo_f, w2_f,
            wq_sum, w1_sum, q1, p1, inv1, x_v, b1_v, b2_v, xs, b1s, b2s, k_sem, v_sem, w_sem):
    do_dma = opts.get("dma", True)
    do_cmp = opts.get("cmp", True)
    nwo = opts.get("nwo", 19)
    nw2 = opts.get("nw2", 8)
    k_src = k_hbm.bitcast(U32)
    v_src = v_hbm.bitcast(U32)
    row8 = lax.broadcasted_iota(jnp.int32, (G, 128), 0)

    def start_kv(src, dst, sem, b, g, n, base=0):
        row = (n % 2) * (W // 4) + (n // 2) * ROWS + base
        if not isinstance(row, int):
            row = pl.multiple_of(row, ROWS)
        if do_dma:
            pltpu.make_async_copy(
                src.at[b, pl.ds(g * G, G), pl.ds((SK - W) // 2 + row, ROWS), :],
                dst.at[pl.ds(g * G, G), pl.ds(row, ROWS), :], sem).start(priority=n % 2)

    def wait(view, sem):
        if do_dma:
            pltpu.make_async_copy(view, view, sem).wait()

    small = [pltpu.make_async_copy(s, d, w_sem.at[0])
             for s, d in ((x_hbm, x_v), (b1_hbm, b1_v), (b2_hbm, b2_v))]

    def start_weight(src, dst, sem, queue, lead, row, col):
        idx = (lead, pl.ds(row if isinstance(row, int) else pl.multiple_of(row, 8), 8), col)
        pltpu.make_async_copy(src.at[idx], dst.reshape(src.shape).at[idx], sem).start(priority=queue)

    halves = (pl.ds(0, 384), pl.ds(384, 256))

    def start_wo(row):
        for col in halves:
            for queue in range(2):
                start_weight(wo_hbm, wo_v, w_sem.at[1], queue, slice(None), queue * 512 + row, col)

    def start_mlp(row):
        for col in halves:
            start_weight(w1_hbm, w1_v, w_sem.at[1], 0, slice(None), row, col)
            start_weight(w2_hbm, w2_v, w_sem.at[1], 1, slice(None), row, col)

    @pl.loop(0, 8)
    def _(i):
        for c in range(8):
            for queue in range(2):
                start_weight(wq_hbm, wq_v, w_sem.at[0], queue, pl.ds(queue * 5, 5), i * 8,
                             pl.ds(c * 512, 512))

    for c in small:
        c.start()
    pl.loop(0, 16)(lambda i: start_wo(i * 8))
    for c in small:
        c.wait()
    pltpu.make_async_copy(wq_v, wq_v, w_sem.at[0]).wait()

    xs[...] = x_v[...].astype(F32)
    b2s[...] = jnp.broadcast_to(b2_v[...].astype(F32).reshape(1, D), (G, D))
    b1 = jnp.concatenate([b1_v[...].astype(F32).reshape(1, F),
                          jnp.zeros((1, NF * 128 - F), F32)], axis=1)
    for f in range(NF):
        b1s[f] = jnp.broadcast_to(b1[:, f * 128:(f + 1) * 128], (G, 128))
    ones = jnp.ones((G, D), BF16)

    m1, _, v1 = _moments(xs[...])
    y1 = ((xs[...] - m1) * lax.rsqrt(v1 + EPS)).astype(BF16)

    @pl.loop(0, 2 * NG)
    def _(step):
        g = step // 2
        for n in range(6):
            start_wo((16 + step * 6 + n) * 8)
            start_mlp((step * 6 + n) * 8)

        @pl.when(step % 2 == 0)
        def _():
            for j in range(G):
                col = pl.ds(pl.multiple_of((g * G + j) * DH, DH), DH)
                q1[pl.ds(g * G + j, B, stride=H), :] = jnp.dot(
                    y1, wq_v[:, col], preferred_element_type=F32)
                for n in range(ND):
                    blk = wq_v[n * 128:(n + 1) * 128, col].astype(F32)
                    kt[0, n, pl.ds(j, DH, stride=G), :] = blk.T

        @pl.when(step % 2 == 1)
        def _():
            for u in range(G):
                blk = jnp.concatenate([kt[0, n, u * 128:(u + 1) * 128, :].T for n in range(ND)],
                                      axis=0).astype(BF16)
                wq_p[g * G + u] = pltpu.bitcast(blk, U32)
                wq_sum[g * G + u] = jnp.dot(ones, blk, preferred_element_type=F32)

    for n in range(48, F // 32):
        start_mlp(n * 8)
    for n in range(NCOPY):
        start_kv(k_src, kbuf, k_sem.at[0], 0, 0, n)
    for buf in (wo_v, w1_v, w2_v):
        pltpu.make_async_copy(buf, buf, w_sem.at[1]).wait()

    @pl.loop(0, G)
    def _(i):
        for n in range(16):
            start_kv(k_src, kbuf, k_sem.at[1 + i // 4], 0, 1 + i // 4, n, (i % 4) * 8 * ROWS)
        for u in range(H // G):
            h = i * (H // G) + u
            blk = wo_v[pl.ds(pl.multiple_of(h * DH, DH), DH), :]
            wo_f[h] = blk.astype(F32)
            for n in range(ND):
                wo_p[h, n] = pltpu.bitcast(blk[:, n * 128:(n + 1) * 128], U32)

    def retile_mlp(f, a, b):
        a = jnp.concatenate([a[:, n * 128:(n + 1) * 128].T for n in range(ND)], axis=0)
        w1_p[f] = pltpu.bitcast(a, U32)
        w1_sum[f] = jnp.dot(ones, a, preferred_element_type=F32)
        w2_f[f] = b.astype(F32)
        for n in range(ND):
            w2_p[f, n] = pltpu.bitcast(b[:, n * 128:(n + 1) * 128], U32)

    @pl.loop(0, F // 128)
    def _(f):
        @pl.when((f >= 2) & (f < 10))
        def _():
            for n in range(8):
                start_kv(k_src, kbuf, k_sem.at[3], 0, 3, n, (f - 2) * 4 * ROWS)
        rows = pl.ds(pl.multiple_of(f * 128, 128), 128)
        retile_mlp(f, w1_v[rows, :], w2_v[rows, :])

    pad = jnp.zeros((NF * 128 - F, D), BF16)
    tail = pl.ds(F // 128 * 128, F % 128)
    retile_mlp(NF - 1, jnp.concatenate([w1_v[tail, :], pad], axis=0),
               jnp.concatenate([w2_v[tail, :], pad], axis=0))

    def wait_keys(g):
        wait(kbuf.at[pl.ds(g * G, G)], k_sem.at[g])

    wait_keys(0)
    wait_keys(1)
    if opts.get("pro"):
        wait_keys(2)
        wait_keys(3)
        r = xs[...]
        live = opts["pro"]
        i = pl.multiple_of(lax.fori_loop(0, 2, lambda i, c: c + i, 0) - 1, 8)
        if "q" in live: r = r + jnp.concatenate([pltpu.bitcast(wq_p[i, :8], F32), wq_sum[i], q1[pl.ds(i, 8)], wq_sum[i], wq_sum[i]], axis=1)
        if "o" in live: r = r + wo_f[i, :8] + jnp.concatenate([pltpu.bitcast(wo_p[i, 0, :8], F32)] * 5, axis=1)
        if "m" in live: r = r + w2_f[i, :8] + jnp.concatenate([pltpu.bitcast(w2_p[i, 0, :8], F32), pltpu.bitcast(w1_p[i, :8], F32), w1_sum[i], w1_sum[i], w1_sum[i]], axis=1)
        o_ref[...] = r.astype(o_ref.dtype)
        return

    def softmax(score, scale):
        top = jnp.max(functools.reduce(jnp.maximum, score), axis=-1, keepdims=True)
        e = [jnp.exp2((s - top) * scale) for s in score]
        total = jnp.sum(functools.reduce(jnp.add, e), axis=-1, keepdims=True)
        return e, 1.0 / total

    def keys_arrived(b, g):
        q = q1[pl.ds(pl.multiple_of(b * H + g * G, G), G), :].astype(BF16)
        score = [None] * NT
        for j in range(G):
            for t in range(NT):
                blk = _bf(kbuf[g * G + j, t * 64:(t + 1) * 64, :])
                s = lax.dot_general(q, blk, (((1,), (1,)), ((), ())), preferred_element_type=F32)
                score[t] = s if j == 0 else jnp.where(row8 == j, s, score[t])
                kt[g, t, pl.ds(j, DH, stride=G), :] = blk.astype(F32).T
        e, inv = softmax(score, QSCALE)
        p1[g] = jnp.concatenate(e, axis=1)
        inv1[g] = jnp.broadcast_to(inv, (G, 128))

    def start_values(b, g, count, base=0):
        sem = v_sem.at[0 if isinstance(g, int) and g == 0 else 1]
        for n in range(count):
            start_kv(v_src, vbuf, sem, b, g, n, base)

    def finish(x, mxu_sum, vpu_sum):
        out = []
        for n in range(ND):
            r = x[:, n * 128:(n + 1) * 128]
            if vpu_sum[n] is not None:
                r = r + jnp.sum(vpu_sum[n], axis=0, keepdims=True)
            out.append(r + mxu_sum[n])
        return jnp.concatenate(out, axis=1)

    def mlp(x, copies):
        xb = x.astype(BF16)
        m, mc, v = _moments(x)
        r1 = lax.rsqrt(v + EPS)
        r2 = lax.rsqrt(r1 * r1 * (v - mc * mc) + EPS)
        scale, shift = r1 * r2, m + mc
        hid = {}
        mxu_sum, vpu_sum = [None] * ND, [None] * ND

        def up(f):
            h = jnp.dot(xb, _bf(w1_p[f]), preferred_element_type=F32)
            hid[f] = _gelu((h - shift * w1_sum[f]) * scale + b1s[f])

        def down_mxu(f):
            hb = hid[f].astype(BF16)
            for n in range(ND):
                term = jnp.dot(hb, _bf(w2_p[f, n]), preferred_element_type=F32)
                mxu_sum[n] = term if mxu_sum[n] is None else mxu_sum[n] + term

        def down_vpu(f):
            vpu_sum[:] = _vpu_dot(lambda i, n: w2_f[f, i * 8:(i + 1) * 8, n * 128:(n + 1) * 128],
                                  _column(hid[f]), vpu_sum)

        _emit([(up, f, 0, 40) for f in range(NF)] + [(down_mxu, f, 0, 40) for f in range(nw2, NF)],
              [(down_vpu, f, 250 + 40 * f, 40) for f in range(nw2)], copies)
        return finish(x + b2s[...], mxu_sum, vpu_sum)

    def attention(x, extra, layer, late=False):
        q, score, prob, o = {}, {}, {}, {}
        mxu_sum, vpu_sum = [None] * ND, [None] * ND
        if layer == 1:
            for g in range(NG):
                prob[g] = [p1[g, :, t * 128:(t + 1) * 128].astype(BF16) for t in range(NT)], inv1[g]
        else:
            xb = x.astype(BF16)
            m, _, v = _moments(x)
            scale = lax.rsqrt(v + EPS) * QSCALE

        def query(u):
            q[u] = jnp.dot(xb, _bf(wq_p[u]), preferred_element_type=F32) - m * wq_sum[u]

        def scores(u):
            g, r = divmod(u, G)
            score[g] = _vpu_dot(lambda i, t: kt[g, t, r * 128 + i * 8:r * 128 + (i + 1) * 8, :],
                                _column(q[u]), score.get(g, [None] * NT))
            if r == G - 1:
                e, inv = softmax(score[g], scale)
                prob[g] = [p.astype(BF16) for p in e], inv

        def normalize(h, r):
            r = r * prob[h // G][1]
            o[h] = jnp.broadcast_to(r[h % G:h % G + 1, :], (G, DH))

        def values(h):
            p = jnp.concatenate(prob[h // G][0], axis=1)
            normalize(h, jnp.dot(p, _bf(vbuf[h]), preferred_element_type=F32))

        def late_values(t):
            for u in (t, t + NT // 2):
                wait(vbuf.at[pl.ds(H - G, G), pl.ds(u * 64, 64)], k_sem.at[t])
            for h in range(H - G, H):
                for u in (t, t + NT // 2):
                    r = jnp.dot(prob[NG - 1][0][u], _bf(vbuf[h, u * 64:(u + 1) * 64, :]),
                                preferred_element_type=F32)
                    o[h] = r if u == 0 else o[h] + r
                if t == NT // 2 - 1:
                    normalize(h, o[h])

        def out_mxu(h):
            ob = o[h].astype(BF16)
            for n in range(ND):
                term = jnp.dot(ob, _bf(wo_p[h, n]), preferred_element_type=F32)
                mxu_sum[n] = term if mxu_sum[n] is None else mxu_sum[n] + term

        def out_vpu(h):
            vpu_sum[:] = _vpu_dot(lambda i, n: wo_f[h, i * 8:(i + 1) * 8, n * 128:(n + 1) * 128],
                                  _column(o[h]), vpu_sum)

        if layer == 2:
            mxu = [(query, u, 0, 40) for u in range(H)] + [(values, h, 0, 64) for h in range(H)]
            mxu += [(out_mxu, h, 0, 40) for h in range(nwo, H)]
            vpu = [(scores, u, 100, 66) for u in range(H)]
            vpu += [(out_vpu, h, 1480 + 64 * (h + 1), 40) for h in range(nwo)]
        elif late:
            early, nlast = opts.get("early", 20), opts.get("nlast", 3)
            mxu = [(values, h, 0, 64) for h in range(H - G)]
            mxu += [(out_mxu, h, 0, 40) for h in range(early, H - G)]
            mxu += [(late_values, t, 5000, 128) for t in range(NT // 2)]
            mxu += [(out_mxu, h, 0, 40) for h in range(H - G + nlast, H)]
            vpu = [(out_vpu, h, 200 + 64 * (h + 1), 40) for h in range(early)]
            vpu += [(out_vpu, h, 5512, 40) for h in range(H - G, H - G + nlast)]
        else:
            mxu = [(values, h, 0, 64) for h in range(H)] + [(out_mxu, h, 0, 40) for h in range(28, H)]
            vpu = [(out_vpu, h, 200 + 64 * (h + 1), 40) for h in range(28)]
        _emit(mxu, vpu, extra)
        return finish(x, mxu_sum, vpu_sum)

    @pl.loop(opts.get('b0', 0), B)
    def _(b):
        def next_keys(lo, hi):
            for n in range(lo, hi):
                start_kv(k_src, kbuf, k_sem.at[n // NCOPY], b + 1, n // NCOPY, n % NCOPY)

        start_values(b, 0, NCOPY)

        @pl.loop(0, NG)
        def _(g):
            pl.when(g >= 2)(lambda: wait_keys(g))
            if do_cmp and opts.get('tr', True):
                keys_arrived(b, g)

            @pl.when(b < B - 1)
            def _():
                @pl.when(g < 2)
                def _():
                    start_values(b, 1 + 2 * g, NCOPY)
                    start_values(b, 2, NCOPY // 2, g * (W // 8))

                pl.when(g == 2)(lambda: next_keys(0, NCOPY))

            @pl.when(b == B - 1)
            def _():
                for step, (lo, hi) in enumerate(((0, 44), (44, 88), (88, 128))):
                    @pl.when(g == step)
                    def _():
                        for n in range(lo, hi):
                            start_kv(v_src, vbuf, v_sem.at[1], B - 1, 1 + n // NCOPY, n % NCOPY)

        @pl.when(b < B - 1)
        def _():
            def burst(g, lo, hi):
                wait_keys(g)
                next_keys(lo, hi)

            c1, c2 = opts.get("cuts", (112, 184))
            next_keys(NCOPY, c1)
            wait(vbuf.at[pl.ds(0, G)], v_sem.at[0])
            wait(vbuf.at[pl.ds(G, H - G)], v_sem.at[1])
            if not do_cmp or not opts.get('lay', True):
                burst(0, c1, c2)
                burst(1, c2, NG * NCOPY)
                return
            x = jnp.broadcast_to(xs[pl.ds(b, 1), :], (G, D))
            x = attention(x, [], 1)
            burst(0, c1, c2)
            x = mlp(x, [])
            x = attention(x, [(lambda _: burst(1, c2, NG * NCOPY), None, opts.get("mid", 2200), 0)], 2)
            xs[pl.ds(b, 1), :] = mlp(x, [])[:1]

    for n in range(NCOPY):
        start_kv(v_src, vbuf, k_sem.at[n // 16], B - 1, NG - 1, n)
    wait(vbuf.at[pl.ds(0, G)], v_sem.at[0])
    wait(vbuf.at[pl.ds(G, 2 * G)], v_sem.at[1])
    x = jnp.broadcast_to(xs[B - 1:, :], (G, D))
    if do_cmp and opts.get('last', True):
        x = mlp(attention(x, [], 1, late=True), [])
        if opts.get("tail", True):
            x = mlp(attention(x, [], 2), [])
    else:
        for u in range(NT):
            wait(vbuf.at[pl.ds(H - G, G), pl.ds(u * 64, 64)], k_sem.at[u % 4])
    rowd = lax.broadcasted_iota(jnp.int32, (B, D), 0)
    o_ref[...] = jnp.where(rowd == B - 1, x, xs[...]).astype(o_ref.dtype)


def make(**opts):
    def fn(A_x, A_k_cache, A_v_cache, A_wq, A_wo, B_x, B_w1, B_b1, B_w2, B_b2):
        del B_x
        any_spec = pl.BlockSpec(memory_space=pl.ANY)
        out = pl.pallas_call(
            functools.partial(_kernel, opts),
            out_shape=jax.ShapeDtypeStruct((B, D), A_x.dtype),
            in_specs=[any_spec] * 9,
            out_specs=pl.BlockSpec(memory_space=pltpu.VMEM),
            scratch_shapes=[
                pltpu.VMEM((H, W // 2, DH), U32),
                pltpu.VMEM((H, W // 2, DH), U32),
                pltpu.VMEM((NG, NT, DH * G, 128), F32),
                pltpu.VMEM((D, H * DH), BF16),
                pltpu.VMEM((H * DH, D), BF16),
                pltpu.VMEM((F, D), BF16),
                pltpu.VMEM((F, D), BF16),
                pltpu.VMEM((H, D // 2, 128), U32),
                pltpu.VMEM((H, ND, DH // 2, 128), U32),
                pltpu.VMEM((NF, D // 2, 128), U32),
                pltpu.VMEM((NF, ND, 64, 128), U32),
                pltpu.VMEM((H, DH, D), F32),
                pltpu.VMEM((NF, 128, D), F32),
                pltpu.VMEM((H, G, 128), F32),
                pltpu.VMEM((NF, G, 128), F32),
                pltpu.VMEM((B * H, DH), F32),
                pltpu.VMEM((NG, G, W), F32),
                pltpu.VMEM((NG, G, 128), F32),
                pltpu.VMEM((B, D), BF16),
                pltpu.VMEM((F,), BF16),
                pltpu.VMEM((D,), BF16),
                pltpu.VMEM((B, D), F32),
                pltpu.VMEM((NF, G, 128), F32),
                pltpu.VMEM((G, D), F32),
                pltpu.SemaphoreType.DMA((NG,)),
                pltpu.SemaphoreType.DMA((2,)),
                pltpu.SemaphoreType.DMA((2,)),
            ],
            compiler_params=pltpu.CompilerParams(
                vmem_limit_bytes=110 * 1024 * 1024, disable_bounds_checks=True,
                flags=opts.get("flags")),
        )(A_x.reshape(B, D), A_k_cache, A_v_cache, A_wq.reshape(10, D // 10, H * DH),
          A_wo.reshape(4, H * DH // 4, D), B_w1.T.reshape(4, F // 4, D), B_b1,
          B_w2.reshape(4, F // 4, D), B_b2)
        return out.reshape(B, 1, D)
    return fn


pallas_interleave_layers__sliding_block_cached__mixer_channel_mlp__decode_kernel = jax.jit(make())
```

```python
import functools

import jax
import jax.numpy as jnp
from jax import lax
import jax.experimental.pallas as pl
import jax.experimental.pallas.tpu as pltpu

BF16 = jnp.bfloat16
F32 = jnp.float32
U32 = jnp.uint32

B, D, H, SK, DH, F = 8, 640, 32, 4096, 128, 1728
W = min(4096, max(256, SK // 4))
G = 8
NG = H // G
ND = D // 128
NF = -(-F // 128)
NT = W // 128
ROWS = 8
NCOPY = W // 2 // ROWS
EPS = 1e-5
QSCALE = (DH ** -0.5) * 1.4426950408889634


def _gelu(x):
    c = 0.7978845608028654
    return 0.5 * x * (1.0 + jnp.tanh(c * (x + 0.044715 * (x * x * x))))


def _bf(x):
    return pltpu.bitcast(x, BF16)


def _moments(x):
    m = jnp.mean(x, axis=-1, keepdims=True)
    c = x - m
    return m, jnp.mean(c, axis=-1, keepdims=True), jnp.mean(c * c, axis=-1, keepdims=True)


def _column(r):
    return jnp.concatenate([r] * 16, axis=0).T


def _vpu_dot(load, col, acc, width=0):
    part = [None] * len(acc)
    width = width or len(acc)
    for t0 in range(0, len(acc), width):
        for i in range(16):
            for t in range(t0, min(len(acc), t0 + width)):
                term = load(i, t) * col[i * 8:(i + 1) * 8, :]
                part[t] = term if i == 0 else part[t] + term
    return [p if a is None else a + p for a, p in zip(acc, part)]


def _emit(*units):
    queues, free, done, plan = [list(u) for u in units], [0] * len(units), {}, []
    while any(queues):
        start, n = min((max([free[n]] + [done[k] + d for k, d in q[0][3].items()]), n)
                       for n, q in enumerate(queues) if q and all(k in done for k in q[0][3]))
        fn, arg, cycles, _ = queues[n].pop(0)
        free[n] = done[fn, arg] = start + cycles
        plan.append((start, len(plan), fn, arg))
    for _, _, fn, arg in sorted(plan, key=lambda t: t[:2]):
        fn(arg)


def _kernel(opts, x_hbm, k_hbm, v_hbm, wq_hbm, wo_hbm, w1_hbm, b1_hbm, w2_hbm, b2_hbm, o_ref,
            kbuf, vbuf, kt, wq_v, wo_v, w1_v, w2_v, wq_p, wo_p, w1_p, w2_p, wo_f, w1_f, w2_f,
            wq_sum, w1_sum, q1, p1, inv1, x_v, b1_v, b2_v, xs, b1s, b2s, k_sem, v_sem, w_sem, fence_sem):
    do_dma = opts.get("dma", True)
    do_cmp = opts.get("cmp", True)
    LATE = opts.get("LATE", ((24, 4, tuple(range(NT))), (28, 4, (0, 1, 2, 3, 4, 5)), (28, 4, (6, 7))))
    k_src = k_hbm.bitcast(U32)
    v_src = v_hbm.bitcast(U32)
    row8 = lax.broadcasted_iota(jnp.int32, (G, 128), 0)

    def start_kv(src, dst, sem, b, g, n, base=0):
        row = (n % 2) * (W // 4) + (n // 2) * ROWS + base
        if not isinstance(row, int):
            row = pl.multiple_of(row, ROWS)
        if do_dma:
            pltpu.make_async_copy(
                src.at[b, pl.ds(g * G, G), pl.ds((SK - W) // 2 + row, ROWS), :],
                dst.at[pl.ds(g * G, G), pl.ds(row, ROWS), :], sem).start(priority=n % 2)

    def wait(view, sem):
        if do_dma:
            pltpu.make_async_copy(view, view, sem).wait()

    small = [pltpu.make_async_copy(s, d, w_sem.at[0])
             for s, d in ((x_hbm, x_v), (b1_hbm, b1_v), (b2_hbm, b2_v))]

    def start_weight(src, dst, sem, queue, lead, row, col):
        if opts.get('now'): return
        idx = (lead, pl.ds(row if isinstance(row, int) else pl.multiple_of(row, 8), 8), col)
        pltpu.make_async_copy(src.at[idx], dst.reshape(src.shape).at[idx], sem).start(priority=queue)

    halves = (pl.ds(0, 384), pl.ds(384, 256))
    if opts.get('nosmall'): small = []

    def start_wo(row):
        for col in halves:
            for queue in range(2):
                start_weight(wo_hbm, wo_v, w_sem.at[1], queue, slice(None), queue * 512 + row, col)

    def start_mlp(row):
        for col in halves:
            start_weight(w1_hbm, w1_v, w_sem.at[1], 0, slice(None), row, col)
            start_weight(w2_hbm, w2_v, w_sem.at[1], 1, slice(None), row, col)

    @pl.loop(0, 8)
    def _(i):
        for c in range(8):
            for queue in range(2):
                start_weight(wq_hbm, wq_v, w_sem.at[0], queue, pl.ds(queue * 5, 5), i * 8,
                             pl.ds(c * 512, 512))

    for c in small:
        c.start()
    pl.loop(0, 16)(lambda i: start_wo(i * 8))
    pl.loop(0, 6)(lambda i: start_mlp(i * 8))
    for c in small:
        c.wait()
    if not opts.get('now'): pltpu.make_async_copy(wq_v, wq_v, w_sem.at[0]).wait()

    xs[...] = x_v[...].astype(F32)
    b2s[...] = jnp.broadcast_to(b2_v[...].astype(F32).reshape(1, D), (G, D))
    b1 = jnp.concatenate([b1_v[...].astype(F32).reshape(1, F),
                          jnp.zeros((1, NF * 128 - F), F32)], axis=1)
    for f in range(NF):
        b1s[f] = jnp.broadcast_to(b1[:, f * 128:(f + 1) * 128], (G, 128))
    ones = jnp.ones((G, D), BF16)

    m1, _, v1 = _moments(xs[...])
    y1 = ((xs[...] - m1) * lax.rsqrt(v1 + EPS)).astype(BF16)

    @pl.loop(0, 2 * NG)
    def _(step):
        g = step // 2

        for n in range(6):
            start_wo((16 + step * 6 + n) * 8)
            start_mlp((6 + step * 6 + n) * 8)

        @pl.when(step % 2 == 0)
        def _():
            for j in range(G if opts.get('jp', 1) else 0):
                col = pl.ds(pl.multiple_of((g * G + j) * DH, DH), DH)
                q1[pl.ds(g * G + j, B, stride=H), :] = jnp.dot(
                    y1, wq_v[:, col], preferred_element_type=F32)
                for n in range(ND):
                    blk = wq_v[n * 128:(n + 1) * 128, col].astype(F32)
                    kt[0, n, pl.ds(j, DH, stride=G), :] = blk.T

        @pl.when(step % 2 == 1)
        def _():
            for u in range(G if opts.get('up', 1) else 0):
                blk = jnp.concatenate([kt[0, n, u * 128:(u + 1) * 128, :].T for n in range(ND)],
                                      axis=0).astype(BF16)
                wq_p[g * G + u] = pltpu.bitcast(blk, U32)
                wq_sum[g * G + u] = jnp.dot(ones, blk, preferred_element_type=F32)

    for n in range(NCOPY):
        start_kv(k_src, kbuf, k_sem.at[0], 0, 0, n)
    for buf in (wo_v, w1_v, w2_v):
        if not opts.get('now'): pltpu.make_async_copy(buf, buf, w_sem.at[1]).wait()

    @pl.loop(0, G)
    def _(i):
        for n in range(16):
            start_kv(k_src, kbuf, k_sem.at[1 + i // 4], 0, 1 + i // 4, n, (i % 4) * 8 * ROWS)
        for u in range(H // G if opts.get('op', 1) else 0):
            h = i * (H // G) + u
            blk = wo_v[pl.ds(pl.multiple_of(h * DH, DH), DH), :]
            wo_f[h] = blk.astype(F32)
            for n in range(ND):
                wo_p[h, n] = pltpu.bitcast(blk[:, n * 128:(n + 1) * 128], U32)

    def retile_mlp(f, a, b):
        if not opts.get('mp', 1): return
        a = jnp.concatenate([a[:, n * 128:(n + 1) * 128].T for n in range(ND)], axis=0)
        w1_p[f] = pltpu.bitcast(a, U32)
        w1_f[f] = a.astype(F32)
        w1_sum[f] = jnp.dot(ones, a, preferred_element_type=F32)
        w2_f[f] = b.astype(F32)
        for n in range(ND):
            w2_p[f, n] = pltpu.bitcast(b[:, n * 128:(n + 1) * 128], U32)

    @pl.loop(0, F // 128)
    def _(f):
        @pl.when((f >= 2) & (f < 10))
        def _():
            for n in range(8):
                start_kv(k_src, kbuf, k_sem.at[3], 0, 3, n, (f - 2) * 4 * ROWS)
        rows = pl.ds(pl.multiple_of(f * 128, 128), 128)
        retile_mlp(f, w1_v[rows, :], w2_v[rows, :])

    pad = jnp.zeros((NF * 128 - F, D), BF16)
    tail = pl.ds(F // 128 * 128, F % 128)
    retile_mlp(NF - 1, jnp.concatenate([w1_v[tail, :], pad], axis=0),
               jnp.concatenate([w2_v[tail, :], pad], axis=0))

    def wait_keys(g):
        wait(kbuf.at[pl.ds(g * G, G)], k_sem.at[g])

    wait_keys(0)
    wait_keys(1)
    if opts.get("pro"):
        wait_keys(2)
        wait_keys(3)
        r = xs[...]
        live = opts["pro"]
        i = pl.multiple_of(lax.fori_loop(0, 2, lambda i, c: c + i, 0) - 1, 8)
        if "q" in live: r = r + jnp.concatenate([pltpu.bitcast(wq_p[i, :8], F32), wq_sum[i], q1[pl.ds(i, 8)], wq_sum[i], wq_sum[i]], axis=1)
        if "o" in live: r = r + wo_f[i, :8] + jnp.concatenate([pltpu.bitcast(wo_p[i, 0, :8], F32)] * 5, axis=1)
        if "m" in live: r = r + w2_f[i, :8] + jnp.concatenate([pltpu.bitcast(w2_p[i, 0, :8], F32), pltpu.bitcast(w1_p[i, :8], F32), w1_sum[i], w1_sum[i], w1_sum[i]], axis=1)
        o_ref[...] = r.astype(o_ref.dtype)
        return

    def softmax(score, scale):
        top = jnp.max(functools.reduce(jnp.maximum, score), axis=-1, keepdims=True)
        e = [jnp.exp2((s - top) * scale) for s in score]
        total = jnp.sum(functools.reduce(jnp.add, e), axis=-1, keepdims=True)
        return e, 1.0 / total

    def keys_arrived(b, g):
        q = q1[pl.ds(pl.multiple_of(b * H + g * G, G), G), :].astype(BF16)
        score = [None] * NT
        for j in range(G):
            for t in range(NT):
                blk = _bf(kbuf[g * G + j, t * 64:(t + 1) * 64, :])
                s = lax.dot_general(q, blk, (((1,), (1,)), ((), ())), preferred_element_type=F32)
                score[t] = s if j == 0 else jnp.where(row8 == j, s, score[t])
                kt[g, t, pl.ds(j, DH, stride=G), :] = blk.astype(F32).T
        e, inv = softmax(score, QSCALE)
        p1[g] = jnp.concatenate(e, axis=1)
        inv1[g] = jnp.broadcast_to(inv, (G, 128))

    def start_values(b, g, count, base=0):
        sem = v_sem.at[0]
        for n in range(count):
            start_kv(v_src, vbuf, sem, b, g, n, base)

    def finish(x, mxu_sum, vpu_sum):
        out = []
        for n in range(ND):
            r = x[:, n * 128:(n + 1) * 128]
            if vpu_sum[n] is not None:
                r = r + jnp.sum(vpu_sum[n], axis=0, keepdims=True)
            out.append(r + mxu_sum[n])
        return jnp.concatenate(out, axis=1)

    def mlp(x, cfg):
        nw1, nw2 = cfg.get("nw1", 4), cfg.get("nw2", 6)
        xb = x.astype(BF16)
        m, mc, v = _moments(x)
        r1 = lax.rsqrt(v + EPS)
        r2 = lax.rsqrt(r1 * r1 * (v - mc * mc) + EPS)
        scale, shift = r1 * r2, m + mc
        hid = {}
        mxu_sum, vpu_sum, pre = [None] * ND, [None] * ND, [None] * nw1

        def activate(f, h):
            hid[f] = _gelu((h - shift * w1_sum[f]) * scale + b1s[f])

        def up_mxu(f):
            activate(f, jnp.dot(xb, _bf(w1_p[f]), preferred_element_type=F32))

        def up_vpu(n):
            pre[:] = _vpu_dot(lambda i, t: w1_f[NF - nw1 + t, n * 128 + i * 8:n * 128 + (i + 1) * 8, :],
                              _column(x[:, n * 128:(n + 1) * 128]), pre, cfg.get("vm1", 0))
            if n == ND - 1:
                for t in range(nw1):
                    activate(NF - nw1 + t, jnp.broadcast_to(
                        jnp.sum(pre[t], axis=0, keepdims=True), (G, 128)))

        def down_mxu(f):
            hb = hid[f].astype(BF16)
            for n in range(ND):
                term = jnp.dot(hb, _bf(w2_p[f, n]), preferred_element_type=F32)
                mxu_sum[n] = term if mxu_sum[n] is None else mxu_sum[n] + term

        def down_vpu(f):
            vpu_sum[:] = _vpu_dot(lambda i, n: w2_f[f, i * 8:(i + 1) * 8, n * 128:(n + 1) * 128],
                                  _column(hid[f]), vpu_sum, cfg.get("vm1", 0))

        made = lambda f: {(up_mxu, f): cfg.get("m0", 200)} if f < NF - nw1 else {(up_vpu, ND - 1): 80}
        _emit([(up_mxu, f, 40, {}) for f in range(NF - nw1)]
              + [(down_mxu, f, 40, made(f)) for f in range(nw2, NF)],
              [(up_vpu, n, 8 * nw1, {}) for n in range(ND if nw1 else 0)]
              + [(down_vpu, f, 40, made(f)) for f in range(nw2)])
        return finish(x + b2s[...], mxu_sum, vpu_sum)

    def attention(x, layer, cfg, extra=()):
        q, score, prob, o = {}, {}, {}, {}
        mxu_sum, vpu_sum = [None] * ND, [None] * ND
        if layer == 1:
            for g in range(NG):
                prob[g] = [p1[g, :, t * 128:(t + 1) * 128].astype(BF16) for t in range(NT)], inv1[g]
        else:
            xb = x.astype(BF16)
            m, _, v = _moments(x)
            scale = lax.rsqrt(v + EPS) * QSCALE

        def query(u):
            q[u] = jnp.dot(xb, _bf(wq_p[u]), preferred_element_type=F32) - m * wq_sum[u]

        def scores(u):
            g, r = divmod(u, G)
            score[g] = _vpu_dot(lambda i, t: kt[g, t, r * 128 + i * 8:r * 128 + (i + 1) * 8, :],
                                _column(q[u]), score.get(g, [None] * NT), cfg.get("vm", 0))

        def probs(g):
            e, inv = softmax(score[g], scale)
            prob[g] = [p.astype(BF16) for p in e], inv

        def weigh(h, tiles, step):
            for t in tiles[::step]:
                p = jnp.concatenate(prob[h // G][0][t:t + step], axis=1)
                r = jnp.dot(p, _bf(vbuf[h, t * 64:(t + step) * 64, :]), preferred_element_type=F32)
                o[h] = o[h] + r if h in o else r

        def normalize(h):
            r = o[h] * prob[h // G][1]
            o[h] = jnp.broadcast_to(r[h % G:h % G + 1, :], (G, DH))

        def values(h):
            weigh(h, range(NT), cfg.get("pk", 8))
            normalize(h)

        def late_values(n):
            h0, heads, tiles = LATE[n]
            for t in tiles:
                wait(vbuf.at[pl.ds(h0, heads), pl.ds(t * 64, 64)], k_sem.at[n])
            for h in range(h0, h0 + heads):
                weigh(h, tiles, 1)
                if tiles[-1] == NT - 1:
                    normalize(h)

        def out_mxu(h):
            ob = o[h].astype(BF16)
            for n in range(ND):
                term = jnp.dot(ob, _bf(wo_p[h, n]), preferred_element_type=F32)
                mxu_sum[n] = term if mxu_sum[n] is None else mxu_sum[n] + term

        def out_vpu(h):
            vpu_sum[:] = _vpu_dot(lambda i, n: wo_f[h, i * 8:(i + 1) * 8, n * 128:(n + 1) * 128],
                                  _column(o[h]), vpu_sum, cfg.get("vm", 0))

        lq, lp, lo, lv = cfg.get("lat", (200, 100, 120, 120))
        if layer == 2:
            nwo, nlast, pos, lag = cfg.get("nwo", 18), cfg.get("nl", 0), cfg.get("pos", 3), cfg.get("sd", 1)
            weighted = [(values, h, 64, {(probs, h // G): lp}) for h in range(H)]
            mxu = [(query, u, 40, {}) for u in range(H)] + weighted[:pos * G]
            mxu += [(out_mxu, h, 40, {(values, h): lo}) for h in range(nwo, H - G)] + weighted[pos * G:]
            mxu += [(out_mxu, h, 40, {(values, h): lo}) for h in range(max(nwo, H - G + nlast), H)]
            vpu = []
            for u in range(H):
                vpu.append((scores, u, cfg.get("cqk", 60), {(query, u): lq}))
                if u >= lag and (u - lag) % G == G - 1:
                    vpu.append((probs, (u - lag) // G, 16, {}))
            if lag:
                vpu.append((probs, NG - 1, 16, {}))
            vpu += [(out_vpu, h, cfg.get("cwo", 42), {(values, h): lv})
                    for h in [*range(nwo), *range(H - G, H - G + nlast)]]
        elif cfg.get("late"):
            early = cfg.get("early", 16)

            def arrived(_):
                wait(vbuf.at[pl.ds(2 * G, G)], v_sem.at[1])

            mxu = [(values, h, 64, {}) for h in range(2 * G)] + [(arrived, None, 0, {})]
            mxu += [(values, h, 64, {}) for h in range(2 * G, H - G)]
            mxu += [(out_mxu, h, 40, {}) for h in range(early, H - G)]
            for n, (h0, heads, tiles) in enumerate(LATE):
                mxu.append((late_values, n, 128, {(out_vpu, early - 1): 0}))
                if tiles[-1] == NT - 1:
                    mxu += [(out_mxu, h, 40, {}) for h in range(h0, h0 + heads)]
            vpu = [(out_vpu, h, 40, {(values, h): lv}) for h in range(early)]
        else:
            mxu = [(values, h, 64, {}) for h in range(H)] + [(out_mxu, h, 40, {}) for h in range(28, H)]
            vpu = [(out_vpu, h, 40, {(values, h): lv}) for h in range(28)]
        _emit(mxu, vpu, extra)
        return finish(x, mxu_sum, vpu_sum)

    @pl.loop(opts.get('b0', 0), B)
    def _(b):
        def next_keys(lo, hi):
            for n in range(lo, hi):
                start_kv(k_src, kbuf, k_sem.at[n // NCOPY], b + 1, n // NCOPY, n % NCOPY)

        start_values(b, 0, NCOPY)

        @pl.loop(0, NG)
        def _(g):
            pl.when(g >= 2)(lambda: wait_keys(g))
            if do_cmp and opts.get('tr', True):
                keys_arrived(b, g)

            def more_values(cuts):
                for step in range(len(cuts) - 1):
                    @pl.when(g == step)
                    def _():
                        for n in range(cuts[step], cuts[step + 1]):
                            start_kv(v_src, vbuf, v_sem.at[min(n // NCOPY, 1)], b, 1 + n // NCOPY, n % NCOPY)

            @pl.when(b < B - 1)
            def _():
                more_values((0, 96, 192))
                pl.when(g == 2)(lambda: next_keys(0, NCOPY))

            pl.when(b == B - 1)(lambda: more_values((0, 44, 88, 128)))

        @pl.when(b < B - 1)
        def _():
            def burst(g, lo, hi):
                wait_keys(g)
                next_keys(lo, hi)

            c1, c2 = opts.get("cuts", (112, 184))
            next_keys(NCOPY, c1)
            wait(vbuf.at[pl.ds(0, 2 * G)], v_sem.at[0])
            wait(vbuf.at[pl.ds(2 * G, 2 * G)], v_sem.at[1])
            if not do_cmp or not opts.get('lay', True):
                burst(0, c1, c2)
                burst(1, c2, NG * NCOPY)
                return
            x = jnp.broadcast_to(xs[pl.ds(b, 1), :], (G, D))
            x = attention(x, 1, {})
            burst(0, c1, c2)
            x = mlp(x, {})
            halfway = [(lambda _: None, None, opts.get("mid", 1700), {}),
                       (lambda _: burst(1, c2, NG * NCOPY), None, 0, {})]
            xs[pl.ds(b, 1), :] = mlp(attention(x, 2, {}, halfway), {})[:1]

    part = {(h0, t): n for n, (h0, _, tiles) in enumerate(LATE) for t in tiles}
    for h0, heads in dict.fromkeys(p[:2] for p in LATE):
        rows = G * ROWS // heads
        for r in range(0, W // 4, rows):
            for queue in range(2):
                row = queue * (W // 4) + r
                if do_dma:
                    pltpu.make_async_copy(
                        v_src.at[B - 1, pl.ds(h0, heads), pl.ds((SK - W) // 2 + row, rows), :],
                        vbuf.at[pl.ds(h0, heads), pl.ds(row, rows), :],
                        k_sem.at[part[h0, row // 64]]).start(priority=queue)
    wait(vbuf.at[pl.ds(0, 2 * G)], v_sem.at[0])
    x = jnp.broadcast_to(xs[B - 1:, :], (G, D))
    if do_cmp and opts.get('last', True):
        def fence(n):
            if n in opts.get("fence", (0, 2)):
                pl.semaphore_signal(fence_sem, 1)
                pl.semaphore_wait(fence_sem, 1)

        x = attention(x, 1, dict(opts.get("a1", {}), late=True))
        fence(0)
        x = mlp(x, opts.get("m1", {}))
        if opts.get("tail", True):
            fence(1)
            x = attention(x, 2, opts.get("a2", {}))
            fence(2)
            x = mlp(x, opts.get("m2", {}))
    else:
        wait(vbuf.at[pl.ds(2 * G, G)], v_sem.at[1])
        for n, (h0, heads, tiles) in enumerate(LATE):
            for t in tiles:
                wait(vbuf.at[pl.ds(h0, heads), pl.ds(t * 64, 64)], k_sem.at[n])
    rowd = lax.broadcasted_iota(jnp.int32, (B, D), 0)
    o_ref[...] = jnp.where(rowd == B - 1, x, xs[...]).astype(o_ref.dtype)


def make(**opts):
    def fn(A_x, A_k_cache, A_v_cache, A_wq, A_wo, B_x, B_w1, B_b1, B_w2, B_b2):
        del B_x
        any_spec = pl.BlockSpec(memory_space=pl.ANY)
        out = pl.pallas_call(
            functools.partial(_kernel, opts),
            out_shape=jax.ShapeDtypeStruct((B, D), A_x.dtype),
            in_specs=[any_spec] * 9,
            out_specs=pl.BlockSpec(memory_space=pltpu.VMEM),
            scratch_shapes=[
                pltpu.VMEM((H, W // 2, DH), U32),
                pltpu.VMEM((H, W // 2, DH), U32),
                pltpu.VMEM((NG, NT, DH * G, 128), F32),
                pltpu.VMEM((D, H * DH), BF16),
                pltpu.VMEM((H * DH, D), BF16),
                pltpu.VMEM((F, D), BF16),
                pltpu.VMEM((F, D), BF16),
                pltpu.VMEM((H, D // 2, 128), U32),
                pltpu.VMEM((H, ND, DH // 2, 128), U32),
                pltpu.VMEM((NF, D // 2, 128), U32),
                pltpu.VMEM((NF, ND, 64, 128), U32),
                pltpu.VMEM((H, DH, D), F32),
                pltpu.VMEM((NF, D, 128), F32),
                pltpu.VMEM((NF, 128, D), F32),
                pltpu.VMEM((H, G, 128), F32),
                pltpu.VMEM((NF, G, 128), F32),
                pltpu.VMEM((B * H, DH), F32),
                pltpu.VMEM((NG, G, W), F32),
                pltpu.VMEM((NG, G, 128), F32),
                pltpu.VMEM((B, D), BF16),
                pltpu.VMEM((F,), BF16),
                pltpu.VMEM((D,), BF16),
                pltpu.VMEM((B, D), F32),
                pltpu.VMEM((NF, G, 128), F32),
                pltpu.VMEM((G, D), F32),
                pltpu.SemaphoreType.DMA((NG,)),
                pltpu.SemaphoreType.DMA((2,)),
                pltpu.SemaphoreType.DMA((2,)),
                pltpu.SemaphoreType.REGULAR,
            ],
            compiler_params=pltpu.CompilerParams(
                vmem_limit_bytes=110 * 1024 * 1024, disable_bounds_checks=True,
                flags=opts.get("flags")),
        )(A_x.reshape(B, D), A_k_cache, A_v_cache, A_wq.reshape(10, D // 10, H * DH),
          A_wo.reshape(4, H * DH // 4, D), B_w1.T.reshape(4, F // 4, D), B_b1,
          B_w2.reshape(4, F // 4, D), B_b2)
        return out.reshape(B, 1, D)
    return fn


pallas_interleave_layers__sliding_block_cached__mixer_channel_mlp__decode_kernel = jax.jit(make())
```

```python
import functools

import jax
import jax.numpy as jnp
from jax import lax
import jax.experimental.pallas as pl
import jax.experimental.pallas.tpu as pltpu

BF16 = jnp.bfloat16
F32 = jnp.float32
U32 = jnp.uint32

B, D, H, SK, DH, F = 8, 640, 32, 4096, 128, 1728
W = min(4096, max(256, SK // 4))
G = 8
NG = H // G
ND = D // 128
NF = -(-F // 128)
NT = W // 128
ROWS = 8
NCOPY = W // 2 // ROWS
EPS = 1e-5
QSCALE = (DH ** -0.5) * 1.4426950408889634


def _gelu(x):
    c = 0.7978845608028654
    return 0.5 * x * (1.0 + jnp.tanh(c * (x + 0.044715 * (x * x * x))))


def _bf(x):
    return pltpu.bitcast(x, BF16)


def _moments(x):
    m = jnp.mean(x, axis=-1, keepdims=True)
    c = x - m
    return m, jnp.mean(c, axis=-1, keepdims=True), jnp.mean(c * c, axis=-1, keepdims=True)


def _column(r):
    return jnp.concatenate([r] * 16, axis=0).T


def _vpu_dot(load, col, acc, width=0):
    part = [None] * len(acc)
    width = width or len(acc)
    for t0 in range(0, len(acc), width):
        for i in range(16):
            for t in range(t0, min(len(acc), t0 + width)):
                term = load(i, t) * col[i * 8:(i + 1) * 8, :]
                part[t] = term if i == 0 else part[t] + term
    return [p if a is None else a + p for a, p in zip(acc, part)]


def _emit(*units):
    queues, free, done, plan = [list(u) for u in units], [0] * len(units), {}, []
    while any(queues):
        start, n = min((max([free[n]] + [done[k] + d for k, d in q[0][3].items()]), n)
                       for n, q in enumerate(queues) if q and all(k in done for k in q[0][3]))
        fn, arg, cycles, _ = queues[n].pop(0)
        free[n] = done[fn, arg] = start + cycles
        plan.append((start, len(plan), fn, arg))
    for _, _, fn, arg in sorted(plan, key=lambda t: t[:2]):
        fn(arg)


def _kernel(opts, x_hbm, k_hbm, v_hbm, wq_hbm, wo_hbm, w1_hbm, b1_hbm, w2_hbm, b2_hbm, o_ref,
            kbuf, vbuf, kt, wq_v, wo_v, w1_v, w2_v, wq_p, wo_p, w1_p, w2_p, wo_f, w1_f, w2_f,
            wq_sum, w1_sum, q1, p1, inv1, x_v, b1_v, b2_v, xs, b1s, b2s, k_sem, v_sem, w_sem, fence_sem):
    do_dma = opts.get("dma", True)
    do_cmp = opts.get("cmp", True)
    LATE = opts.get("LATE", ((24, 4, tuple(range(NT))), (28, 4, (0, 1, 2, 3, 4, 5)), (28, 4, (6, 7))))
    k_src = k_hbm.bitcast(U32)
    v_src = v_hbm.bitcast(U32)
    row8 = lax.broadcasted_iota(jnp.int32, (G, 128), 0)

    def start_kv(src, dst, sem, b, g, n, base=0):
        nh = opts.get("nh", 2)
        step, part = divmod(n // 2, G // nh)
        row = (n % 2) * (W // 4) + step * (G * ROWS // nh) + base
        if not isinstance(row, int):
            row = pl.multiple_of(row, ROWS)
        if do_dma:
            pltpu.make_async_copy(
                src.at[b, pl.ds(g * G + part * nh, nh), pl.ds((SK - W) // 2 + row, G * ROWS // nh), :],
                dst.at[pl.ds(g * G + part * nh, nh), pl.ds(row, G * ROWS // nh), :], sem).start(priority=n % 2)

    def wait(view, sem):
        if do_dma:
            pltpu.make_async_copy(view, view, sem).wait()

    small = [pltpu.make_async_copy(s, d, w_sem.at[0])
             for s, d in ((x_hbm, x_v), (b1_hbm, b1_v), (b2_hbm, b2_v))]

    def start_weight(src, dst, sem, queue, lead, row, col):
        if opts.get('now'): return
        idx = (lead, pl.ds(row if isinstance(row, int) else pl.multiple_of(row, 8), 8), col)
        pltpu.make_async_copy(src.at[idx], dst.reshape(src.shape).at[idx], sem).start(priority=queue)

    halves = (pl.ds(0, 384), pl.ds(384, 256))
    if opts.get('nosmall'): small = []

    def start_wo(row):
        for col in halves:
            for queue in range(2):
                start_weight(wo_hbm, wo_v, w_sem.at[1], queue, slice(None), queue * 512 + row, col)

    def start_mlp(row):
        for col in halves:
            start_weight(w1_hbm, w1_v, w_sem.at[1], 0, slice(None), row, col)
            start_weight(w2_hbm, w2_v, w_sem.at[1], 1, slice(None), row, col)

    @pl.loop(0, 8)
    def _(i):
        for c in range(8):
            for queue in range(2):
                start_weight(wq_hbm, wq_v, w_sem.at[0], queue, pl.ds(queue * 5, 5), i * 8,
                             pl.ds(c * 512, 512))

    for c in small:
        c.start()
    pl.loop(0, 16)(lambda i: start_wo(i * 8))
    pl.loop(0, 6)(lambda i: start_mlp(i * 8))
    for c in small:
        c.wait()
    if not opts.get('now'): pltpu.make_async_copy(wq_v, wq_v, w_sem.at[0]).wait()

    xs[...] = x_v[...].astype(F32)
    b2s[...] = jnp.broadcast_to(b2_v[...].astype(F32).reshape(1, D), (G, D))
    b1 = jnp.concatenate([b1_v[...].astype(F32).reshape(1, F),
                          jnp.zeros((1, NF * 128 - F), F32)], axis=1)
    for f in range(NF):
        b1s[f] = jnp.broadcast_to(b1[:, f * 128:(f + 1) * 128], (G, 128))
    ones = jnp.ones((G, D), BF16)

    m1, _, v1 = _moments(xs[...])
    y1 = ((xs[...] - m1) * lax.rsqrt(v1 + EPS)).astype(BF16)

    @pl.loop(0, 2 * NG)
    def _(step):
        g = step // 2

        for n in range(6):
            start_wo((16 + step * 6 + n) * 8)
            start_mlp((6 + step * 6 + n) * 8)

        @pl.when(step % 2 == 0)
        def _():
            for j in range(G if opts.get('jp', 1) else 0):
                col = pl.ds(pl.multiple_of((g * G + j) * DH, DH), DH)
                q1[pl.ds(g * G + j, B, stride=H), :] = jnp.dot(
                    y1, wq_v[:, col], preferred_element_type=F32)
                for n in range(ND):
                    blk = wq_v[n * 128:(n + 1) * 128, col].astype(F32)
                    kt[0, n, pl.ds(j, DH, stride=G), :] = blk.T

        @pl.when(step % 2 == 1)
        def _():
            for u in range(G if opts.get('up', 1) else 0):
                blk = jnp.concatenate([kt[0, n, u * 128:(u + 1) * 128, :].T for n in range(ND)],
                                      axis=0).astype(BF16)
                wq_p[g * G + u] = pltpu.bitcast(blk, U32)
                wq_sum[g * G + u] = jnp.dot(ones, blk, preferred_element_type=F32)

    for n in range(NCOPY):
        start_kv(k_src, kbuf, k_sem.at[0], 0, 0, n)
    for buf in (wo_v, w1_v, w2_v):
        if not opts.get('now'): pltpu.make_async_copy(buf, buf, w_sem.at[1]).wait()

    @pl.loop(0, G)
    def _(i):
        for n in range(16):
            start_kv(k_src, kbuf, k_sem.at[1 + i // 4], 0, 1 + i // 4, n, (i % 4) * 8 * ROWS)
        for u in range(H // G if opts.get('op', 1) else 0):
            h = i * (H // G) + u
            blk = wo_v[pl.ds(pl.multiple_of(h * DH, DH), DH), :]
            wo_f[h] = blk.astype(F32)
            for n in range(ND):
                wo_p[h, n] = pltpu.bitcast(blk[:, n * 128:(n + 1) * 128], U32)

    def retile_mlp(f, a, b):
        if not opts.get('mp', 1): return
        a = jnp.concatenate([a[:, n * 128:(n + 1) * 128].T for n in range(ND)], axis=0)
        w1_p[f] = pltpu.bitcast(a, U32)
        w1_f[f] = a.astype(F32)
        w1_sum[f] = jnp.dot(ones, a, preferred_element_type=F32)
        w2_f[f] = b.astype(F32)
        for n in range(ND):
            w2_p[f, n] = pltpu.bitcast(b[:, n * 128:(n + 1) * 128], U32)

    @pl.loop(0, F // 128)
    def _(f):
        @pl.when((f >= 2) & (f < 10))
        def _():
            for n in range(8):
                start_kv(k_src, kbuf, k_sem.at[3], 0, 3, n, (f - 2) * 4 * ROWS)
        rows = pl.ds(pl.multiple_of(f * 128, 128), 128)
        retile_mlp(f, w1_v[rows, :], w2_v[rows, :])

    pad = jnp.zeros((NF * 128 - F, D), BF16)
    tail = pl.ds(F // 128 * 128, F % 128)
    retile_mlp(NF - 1, jnp.concatenate([w1_v[tail, :], pad], axis=0),
               jnp.concatenate([w2_v[tail, :], pad], axis=0))

    def wait_keys(g):
        wait(kbuf.at[pl.ds(g * G, G)], k_sem.at[g])

    wait_keys(0)
    wait_keys(1)
    if opts.get("pro"):
        wait_keys(2)
        wait_keys(3)
        r = xs[...]
        live = opts["pro"]
        i = pl.multiple_of(lax.fori_loop(0, 2, lambda i, c: c + i, 0) - 1, 8)
        if "q" in live: r = r + jnp.concatenate([pltpu.bitcast(wq_p[i, :8], F32), wq_sum[i], q1[pl.ds(i, 8)], wq_sum[i], wq_sum[i]], axis=1)
        if "o" in live: r = r + wo_f[i, :8] + jnp.concatenate([pltpu.bitcast(wo_p[i, 0, :8], F32)] * 5, axis=1)
        if "m" in live: r = r + w2_f[i, :8] + jnp.concatenate([pltpu.bitcast(w2_p[i, 0, :8], F32), pltpu.bitcast(w1_p[i, :8], F32), w1_sum[i], w1_sum[i], w1_sum[i]], axis=1)
        o_ref[...] = r.astype(o_ref.dtype)
        return

    def softmax(score, scale):
        top = jnp.max(functools.reduce(jnp.maximum, score), axis=-1, keepdims=True)
        e = [jnp.exp2((s - top) * scale) for s in score]
        total = jnp.sum(functools.reduce(jnp.add, e), axis=-1, keepdims=True)
        return e, 1.0 / total

    def keys_arrived(b, g):
        q = q1[pl.ds(pl.multiple_of(b * H + g * G, G), G), :].astype(BF16)
        score = [None] * NT
        for j in range(G):
            for t in range(NT):
                blk = _bf(kbuf[g * G + j, t * 64:(t + 1) * 64, :])
                s = lax.dot_general(q, blk, (((1,), (1,)), ((), ())), preferred_element_type=F32)
                score[t] = s if j == 0 else jnp.where(row8 == j, s, score[t])
                kt[g, t, pl.ds(j, DH, stride=G), :] = blk.astype(F32).T
        e, inv = softmax(score, QSCALE)
        p1[g] = jnp.concatenate(e, axis=1)
        inv1[g] = jnp.broadcast_to(inv, (G, 128))

    def start_values(b, g, count, base=0):
        sem = v_sem.at[0]
        for n in range(count):
            start_kv(v_src, vbuf, sem, b, g, n, base)

    def finish(x, mxu_sum, vpu_sum):
        out = []
        for n in range(ND):
            r = x[:, n * 128:(n + 1) * 128]
            if vpu_sum[n] is not None:
                r = r + jnp.sum(vpu_sum[n], axis=0, keepdims=True)
            out.append(r + mxu_sum[n])
        return jnp.concatenate(out, axis=1)

    def mlp(x, cfg):
        nw1, nw2 = cfg.get("nw1", 4), cfg.get("nw2", 6)
        xb = x.astype(BF16)
        m, mc, v = _moments(x)
        r1 = lax.rsqrt(v + EPS)
        r2 = lax.rsqrt(r1 * r1 * (v - mc * mc) + EPS)
        scale, shift = r1 * r2, m + mc
        hid = {}
        mxu_sum, vpu_sum, pre = [None] * ND, [None] * ND, [None] * nw1

        def activate(f, h):
            hid[f] = _gelu((h - shift * w1_sum[f]) * scale + b1s[f])

        def up_mxu(f):
            activate(f, jnp.dot(xb, _bf(w1_p[f]), preferred_element_type=F32))

        def up_vpu(n):
            pre[:] = _vpu_dot(lambda i, t: w1_f[NF - nw1 + t, n * 128 + i * 8:n * 128 + (i + 1) * 8, :],
                              _column(x[:, n * 128:(n + 1) * 128]), pre, cfg.get("vm1", 0))
            if n == ND - 1:
                for t in range(nw1):
                    activate(NF - nw1 + t, jnp.broadcast_to(
                        jnp.sum(pre[t], axis=0, keepdims=True), (G, 128)))

        def down_mxu(f):
            hb = hid[f].astype(BF16)
            for n in range(ND):
                term = jnp.dot(hb, _bf(w2_p[f, n]), preferred_element_type=F32)
                mxu_sum[n] = term if mxu_sum[n] is None else mxu_sum[n] + term

        def down_vpu(f):
            vpu_sum[:] = _vpu_dot(lambda i, n: w2_f[f, i * 8:(i + 1) * 8, n * 128:(n + 1) * 128],
                                  _column(hid[f]), vpu_sum, cfg.get("vm1", 0))

        made = lambda f: {(up_mxu, f): cfg.get("m0", 200)} if f < NF - nw1 else {(up_vpu, ND - 1): 80}
        _emit([(up_mxu, f, 40, {}) for f in range(NF - nw1)]
              + [(down_mxu, f, 40, made(f)) for f in range(nw2, NF)],
              [(up_vpu, n, 8 * nw1, {}) for n in range(ND if nw1 else 0)]
              + [(down_vpu, f, 40, made(f)) for f in range(nw2)])
        return finish(x + b2s[...], mxu_sum, vpu_sum)

    def attention(x, layer, cfg, extra=()):
        q, score, prob, o = {}, {}, {}, {}
        mxu_sum, vpu_sum = [None] * ND, [None] * ND
        if layer == 1:
            for g in range(NG):
                prob[g] = [p1[g, :, t * 128:(t + 1) * 128].astype(BF16) for t in range(NT)], inv1[g]
        else:
            xb = x.astype(BF16)
            m, _, v = _moments(x)
            scale = lax.rsqrt(v + EPS) * QSCALE

        def query(u):
            q[u] = jnp.dot(xb, _bf(wq_p[u]), preferred_element_type=F32) - m * wq_sum[u]

        def scores(u):
            g, r = divmod(u, G)
            score[g] = _vpu_dot(lambda i, t: kt[g, t, r * 128 + i * 8:r * 128 + (i + 1) * 8, :],
                                _column(q[u]), score.get(g, [None] * NT), cfg.get("vm", 0))

        def probs(g):
            e, inv = softmax(score[g], scale)
            prob[g] = [p.astype(BF16) for p in e], inv

        def weigh(h, tiles, step):
            for t in tiles[::step]:
                p = jnp.concatenate(prob[h // G][0][t:t + step], axis=1)
                r = jnp.dot(p, _bf(vbuf[h, t * 64:(t + step) * 64, :]), preferred_element_type=F32)
                o[h] = o[h] + r if h in o else r

        def normalize(h):
            r = o[h] * prob[h // G][1]
            o[h] = jnp.broadcast_to(r[h % G:h % G + 1, :], (G, DH))

        def values(h):
            weigh(h, range(NT), cfg.get("pk", 8))
            normalize(h)

        def late_values(n):
            h0, heads, tiles = LATE[n]
            for t in tiles:
                wait(vbuf.at[pl.ds(h0, heads), pl.ds(t * 64, 64)], k_sem.at[n])
            for h in range(h0, h0 + heads):
                weigh(h, tiles, 1)
                if tiles[-1] == NT - 1:
                    normalize(h)

        def out_mxu(h):
            ob = o[h].astype(BF16)
            for n in range(ND):
                term = jnp.dot(ob, _bf(wo_p[h, n]), preferred_element_type=F32)
                mxu_sum[n] = term if mxu_sum[n] is None else mxu_sum[n] + term

        def out_vpu(h):
            vpu_sum[:] = _vpu_dot(lambda i, n: wo_f[h, i * 8:(i + 1) * 8, n * 128:(n + 1) * 128],
                                  _column(o[h]), vpu_sum, cfg.get("vm", 0))

        lq, lp, lo, lv = cfg.get("lat", (200, 100, 120, 120))
        if layer == 2:
            nwo, nlast, pos, lag = cfg.get("nwo", 18), cfg.get("nl", 0), cfg.get("pos", 3), cfg.get("sd", 1)
            weighted = [(values, h, 64, {(probs, h // G): lp}) for h in range(H)]
            mxu = [(query, u, 40, {}) for u in range(H)] + weighted[:pos * G]
            mxu += [(out_mxu, h, 40, {(values, h): lo}) for h in range(nwo, H - G)] + weighted[pos * G:]
            mxu += [(out_mxu, h, 40, {(values, h): lo}) for h in range(max(nwo, H - G + nlast), H)]
            vpu = []
            for u in range(H):
                vpu.append((scores, u, cfg.get("cqk", 60), {(query, u): lq}))
                if u >= lag and (u - lag) % G == G - 1:
                    vpu.append((probs, (u - lag) // G, 16, {}))
            if lag:
                vpu.append((probs, NG - 1, 16, {}))
            vpu += [(out_vpu, h, cfg.get("cwo", 42), {(values, h): lv})
                    for h in [*range(nwo), *range(H - G, H - G + nlast)]]
        elif cfg.get("late"):
            early = cfg.get("early", 16)

            def arrived(_):
                wait(vbuf.at[pl.ds(2 * G, G)], v_sem.at[1])

            mxu = [(values, h, 64, {}) for h in range(2 * G)] + [(arrived, None, 0, {})]
            mxu += [(values, h, 64, {}) for h in range(2 * G, H - G)]
            mxu += [(out_mxu, h, 40, {}) for h in range(early, H - G)]
            for n, (h0, heads, tiles) in enumerate(LATE):
                mxu.append((late_values, n, 128, {(out_vpu, early - 1): 0}))
                if tiles[-1] == NT - 1:
                    mxu += [(out_mxu, h, 40, {}) for h in range(h0, h0 + heads)]
            vpu = [(out_vpu, h, 40, {(values, h): lv}) for h in range(early)]
        else:
            mxu = [(values, h, 64, {}) for h in range(H)] + [(out_mxu, h, 40, {}) for h in range(28, H)]
            vpu = [(out_vpu, h, 40, {(values, h): lv}) for h in range(28)]
        _emit(mxu, vpu, extra)
        return finish(x, mxu_sum, vpu_sum)

    @pl.loop(opts.get('b0', 0), B)
    def _(b):
        def next_keys(lo, hi):
            for n in range(lo, hi):
                start_kv(k_src, kbuf, k_sem.at[n // NCOPY], b + 1, n // NCOPY, n % NCOPY)

        start_values(b, 0, NCOPY)

        @pl.loop(0, NG)
        def _(g):
            pl.when(g >= 2)(lambda: wait_keys(g))
            if do_cmp and opts.get('tr', True):
                keys_arrived(b, g)

            def more_values(cuts):
                for step in range(len(cuts) - 1):
                    @pl.when(g == step)
                    def _():
                        for n in range(cuts[step], cuts[step + 1]):
                            start_kv(v_src, vbuf, v_sem.at[min(n // NCOPY, 1)], b, 1 + n // NCOPY, n % NCOPY)

            @pl.when(b < B - 1)
            def _():
                more_values((0, 96, 192))
                pl.when(g == 2)(lambda: next_keys(0, NCOPY))

            pl.when(b == B - 1)(lambda: more_values((0, 44, 88, 128)))

        @pl.when(b < B - 1)
        def _():
            def burst(g, lo, hi):
                wait_keys(g)
                next_keys(lo, hi)

            c1, c2 = opts.get("cuts", (112, 184))
            next_keys(NCOPY, c1)
            wait(vbuf.at[pl.ds(0, 2 * G)], v_sem.at[0])
            wait(vbuf.at[pl.ds(2 * G, 2 * G)], v_sem.at[1])
            if not do_cmp or not opts.get('lay', True):
                burst(0, c1, c2)
                burst(1, c2, NG * NCOPY)
                return
            x = jnp.broadcast_to(xs[pl.ds(b, 1), :], (G, D))
            x = attention(x, 1, {})
            burst(0, c1, c2)
            x = mlp(x, {})
            halfway = [(lambda _: None, None, opts.get("mid", 1700), {}),
                       (lambda _: burst(1, c2, NG * NCOPY), None, 0, {})]
            xs[pl.ds(b, 1), :] = mlp(attention(x, 2, {}, halfway), {})[:1]

    part = {(h0, t): n for n, (h0, _, tiles) in enumerate(LATE) for t in tiles}
    for h0, heads in dict.fromkeys(p[:2] for p in LATE):
        rows = G * ROWS // heads
        for r in range(0, W // 4, rows):
            for queue in range(2):
                row = queue * (W // 4) + r
                if do_dma:
                    pltpu.make_async_copy(
                        v_src.at[B - 1, pl.ds(h0, heads), pl.ds((SK - W) // 2 + row, rows), :],
                        vbuf.at[pl.ds(h0, heads), pl.ds(row, rows), :],
                        k_sem.at[part[h0, row // 64]]).start(priority=queue)
    wait(vbuf.at[pl.ds(0, 2 * G)], v_sem.at[0])
    x = jnp.broadcast_to(xs[B - 1:, :], (G, D))
    if do_cmp and opts.get('last', True):
        def fence(n):
            if n in opts.get("fence", (0, 2)):
                pl.semaphore_signal(fence_sem, 1)
                pl.semaphore_wait(fence_sem, 1)

        x = attention(x, 1, dict(opts.get("a1", {}), late=True))
        fence(0)
        x = mlp(x, opts.get("m1", {}))
        if opts.get("tail", True):
            fence(1)
            x = attention(x, 2, opts.get("a2", {}))
            fence(2)
            x = mlp(x, opts.get("m2", {}))
    else:
        wait(vbuf.at[pl.ds(2 * G, G)], v_sem.at[1])
        for n, (h0, heads, tiles) in enumerate(LATE):
            for t in tiles:
                wait(vbuf.at[pl.ds(h0, heads), pl.ds(t * 64, 64)], k_sem.at[n])
    rowd = lax.broadcasted_iota(jnp.int32, (B, D), 0)
    o_ref[...] = jnp.where(rowd == B - 1, x, xs[...]).astype(o_ref.dtype)


def make(**opts):
    def fn(A_x, A_k_cache, A_v_cache, A_wq, A_wo, B_x, B_w1, B_b1, B_w2, B_b2):
        del B_x
        any_spec = pl.BlockSpec(memory_space=pl.ANY)
        out = pl.pallas_call(
            functools.partial(_kernel, opts),
            out_shape=jax.ShapeDtypeStruct((B, D), A_x.dtype),
            in_specs=[any_spec] * 9,
            out_specs=pl.BlockSpec(memory_space=pltpu.VMEM),
            scratch_shapes=[
                pltpu.VMEM((H, W // 2, DH), U32),
                pltpu.VMEM((H, W // 2, DH), U32),
                pltpu.VMEM((NG, NT, DH * G, 128), F32),
                pltpu.VMEM((D, H * DH), BF16),
                pltpu.VMEM((H * DH, D), BF16),
                pltpu.VMEM((F, D), BF16),
                pltpu.VMEM((F, D), BF16),
                pltpu.VMEM((H, D // 2, 128), U32),
                pltpu.VMEM((H, ND, DH // 2, 128), U32),
                pltpu.VMEM((NF, D // 2, 128), U32),
                pltpu.VMEM((NF, ND, 64, 128), U32),
                pltpu.VMEM((H, DH, D), F32),
                pltpu.VMEM((NF, D, 128), F32),
                pltpu.VMEM((NF, 128, D), F32),
                pltpu.VMEM((H, G, 128), F32),
                pltpu.VMEM((NF, G, 128), F32),
                pltpu.VMEM((B * H, DH), F32),
                pltpu.VMEM((NG, G, W), F32),
                pltpu.VMEM((NG, G, 128), F32),
                pltpu.VMEM((B, D), BF16),
                pltpu.VMEM((F,), BF16),
                pltpu.VMEM((D,), BF16),
                pltpu.VMEM((B, D), F32),
                pltpu.VMEM((NF, G, 128), F32),
                pltpu.VMEM((G, D), F32),
                pltpu.SemaphoreType.DMA((NG,)),
                pltpu.SemaphoreType.DMA((2,)),
                pltpu.SemaphoreType.DMA((2,)),
                pltpu.SemaphoreType.REGULAR,
            ],
            compiler_params=pltpu.CompilerParams(
                vmem_limit_bytes=110 * 1024 * 1024, disable_bounds_checks=True,
                flags=opts.get("flags")),
        )(A_x.reshape(B, D), A_k_cache, A_v_cache, A_wq.reshape(10, D // 10, H * DH),
          A_wo.reshape(4, H * DH // 4, D), B_w1.T.reshape(4, F // 4, D), B_b1,
          B_w2.reshape(4, F // 4, D), B_b2)
        return out.reshape(B, 1, D)
    return fn


pallas_interleave_layers__sliding_block_cached__mixer_channel_mlp__decode_kernel = jax.jit(make())
```

```python
import functools

import numpy as np
import jax
import jax.numpy as jnp
from jax import lax
import jax.experimental.pallas as pl
import jax.experimental.pallas.tpu as pltpu

BF16 = jnp.bfloat16
F32 = jnp.float32
U32 = jnp.uint32

B, D, H, SK, DH, F = 8, 640, 32, 4096, 128, 1728
W = min(4096, max(256, SK // 4))
G = 8
NG = H // G
ND = D // 128
NF = -(-F // 128)
NT = W // 128
NCOPY = 64
VPU_QUERIES = 4
VPU_UP = 4
KEY_BURSTS = (64, 104, 134, 144, 160, 196, 228, 242, 256)
EPS = 1e-5
SCORE_SCALE = DH ** -0.5 * 1.4426950408889634
LAST_PARTS = ((H - 8, 0, NT), (H - 4, 0, NT - 2), (H - 4, NT - 2, NT))


def _gelu(x):
    return 0.5 * x * (1.0 + jnp.tanh(0.7978845608028654 * (x + 0.044715 * (x * x * x))))


def _dot(a, packed):
    return jnp.dot(a, pltpu.bitcast(packed, BF16), preferred_element_type=F32)


def _moments(x):
    mean = jnp.mean(x, axis=-1, keepdims=True)
    c = x - mean
    return mean, jnp.mean(c, axis=-1, keepdims=True), jnp.mean(c * c, axis=-1, keepdims=True)


def _softmax(score, scale):
    top = jnp.max(functools.reduce(jnp.maximum, score), axis=-1, keepdims=True)
    e = [jnp.exp2((s - top) * scale) for s in score]
    return e, 1.0 / jnp.sum(functools.reduce(jnp.add, e), axis=-1, keepdims=True)


def _vpu_dot(row, load, acc):
    column = jnp.concatenate([row] * 16, axis=0).T
    part = [None] * len(acc)
    for i in range(16):
        for t in range(len(acc)):
            term = load(i, t) * column[i * 8:(i + 1) * 8, :]
            part[t] = term if i == 0 else part[t] + term
    return [p if a is None else a + p for a, p in zip(acc, part)]


def _interleave(blocks):
    sublane = lax.broadcasted_iota(jnp.int32, (8, 128), 0)
    words = [pltpu.bitcast(blk.T, U32) for blk in blocks]
    out = []
    for i in range(8):
        w = [word[i * 8:(i + 1) * 8, :] for word in words]
        for k in (4, 2, 1):
            low = (sublane & k) == 0
            for j in range(8):
                if j & k == 0:
                    w[j], w[j + k] = (jnp.where(low, w[j], pltpu.roll(w[j + k], k, 0)),
                                      jnp.where(low, pltpu.roll(w[j], 8 - k, 0), w[j + k]))
        for pair in w:
            out += [pltpu.bitcast(pair << 16, F32), pltpu.bitcast(pair & np.uint32(0xFFFF0000), F32)]
    return out


def _sum_rows(a):
    return jnp.broadcast_to(jnp.sum(a, axis=0, keepdims=True), a.shape)


def _emit(*units):
    queues, free, done, plan = [list(u) for u in units], [0] * len(units), {}, []
    while any(queues):
        start, n = min((max([free[n]] + [done[k] + d for k, d in q[0][3].items()]), n)
                       for n, q in enumerate(queues) if q and all(k in done for k in q[0][3]))
        fn, arg, cycles, _ = queues[n].pop(0)
        free[n] = done[fn, arg] = start + cycles
        plan.append((start, len(plan), fn, arg))
    for _, _, fn, arg in sorted(plan, key=lambda t: t[:2]):
        fn(arg)


def _kernel(x_hbm, k_hbm, v_hbm, wq_hbm, wo_hbm, w1t_hbm, b1_hbm, w2_hbm, b2_hbm, o_ref,
            kt, v_p, wq_p, wo_p, w1_p, w2_p, wq_f, wo_f, w1_f, w2_f, wq_sum, w1_sum, b1s, b2s,
            xs, q1, p1, inv1, kbuf, vbuf, wq_v, wo_v, w1t_v, w2_v, x_v, b1_v, b2_v,
            fence_sem):
    sublane = lax.broadcasted_iota(jnp.int32, (G, 128), 0)

    def fence():
        pl.semaphore_signal(fence_sem, 1)
        pl.semaphore_wait(fence_sem, 1)

    def keys_arrived(b, g):
        q = jnp.zeros((G, DH), F32)
        for j in range(G):
            q = jnp.where(sublane == j, q1[g * G + j, pl.ds(b, 1), :], q)
        q = q.astype(BF16)
        score = [None] * NT
        for t in range(NT):
            blocks = [kbuf[g * G + j, t * 128:(t + 1) * 128, :] for j in range(G)]
            for j, blk in enumerate(blocks):
                s = lax.dot_general(q, blk, (((1,), (1,)), ((), ())), preferred_element_type=F32)
                score[t] = s if j == 0 else jnp.where(sublane == j, s, score[t])
            kt[g, :, t * 128:(t + 1) * 128] = jnp.concatenate(_interleave(blocks), axis=0)
        e, inv = _softmax(score, SCORE_SCALE)
        p1[g] = jnp.concatenate(e, axis=1)
        inv1[g] = jnp.broadcast_to(inv, (G, 128))

    def residual(x, mxu_sum, vpu_sum):
        x = x + jnp.concatenate([_sum_rows(a) for a in vpu_sum], axis=1)
        return x + jnp.concatenate(mxu_sum, axis=1)

    def mlp(x, vpu_down=6):
        first = NF - VPU_UP
        xb = x.astype(BF16)
        mean, mean2, var = _moments(x)
        r1 = lax.rsqrt(var + EPS)
        r2 = lax.rsqrt(r1 * r1 * (var - mean2 * mean2) + EPS)
        shift, scale = mean + mean2, r1 * r2
        hidden = {}
        mxu_sum, vpu_sum, pre = [None] * ND, [None] * ND, [None] * VPU_UP

        def activate(f, h):
            hidden[f] = _gelu((h - shift * w1_sum[f]) * scale + b1s[f])

        def up_mxu(f):
            activate(f, _dot(xb, w1_p[f]))

        def up_vpu(n):
            pre[:] = _vpu_dot(
                x[:, n * 128:(n + 1) * 128],
                lambda i, t: w1_f[n * 128 + i * 8:n * 128 + (i + 1) * 8, t * 128:(t + 1) * 128],
                pre)
            if n == ND - 1:
                for t in range(VPU_UP):
                    activate(first + t, _sum_rows(pre[t]))

        def down_mxu(f):
            hb = hidden[f].astype(BF16)
            for n in range(ND):
                term = _dot(hb, w2_p[f, n])
                mxu_sum[n] = term if mxu_sum[n] is None else mxu_sum[n] + term

        def down_vpu(f):
            vpu_sum[:] = _vpu_dot(
                hidden[f], lambda i, n: w2_f[f, i * 8:(i + 1) * 8, n * 128:(n + 1) * 128],
                vpu_sum)

        def made(f):
            return {(up_mxu, f): 200} if f < first else {(up_vpu, ND - 1): 80}

        _emit([(up_mxu, f, 40, {}) for f in range(first)]
              + [(down_mxu, f, 40, made(f)) for f in range(vpu_down, NF)],
              [(up_vpu, n, 8 * VPU_UP, {}) for n in range(ND)]
              + [(down_vpu, f, 40, made(f)) for f in range(vpu_down)])
        return residual(x + b2s[...], mxu_sum, vpu_sum)

    def attention(x, layer, extra=(), arrived=None):
        q, score, prob, out = {}, {}, {}, {}
        mxu_sum, vpu_sum = [None] * ND, [None] * ND
        pre = [None] * VPU_QUERIES
        if layer == 1:
            for g in range(NG):
                prob[g] = [p1[g, :, t * 128:(t + 1) * 128].astype(BF16) for t in range(NT)], inv1[g]
        else:
            xb = x.astype(BF16)
            mean, _, var = _moments(x)
            scale = lax.rsqrt(var + EPS) * SCORE_SCALE

        def query(u):
            q[u] = _dot(xb, wq_p[u]) - mean * wq_sum[u]

        def query_vpu(n):
            pre[:] = _vpu_dot(
                x[:, n * 128:(n + 1) * 128],
                lambda i, t: wq_f[n * 128 + i * 8:n * 128 + (i + 1) * 8, t * 128:(t + 1) * 128],
                pre)
            if n == ND - 1:
                for t, u in enumerate(range(H - VPU_QUERIES, H)):
                    q[u] = _sum_rows(pre[t]) - mean * wq_sum[u]

        def scores(u):
            g, r = divmod(u, G)
            score[g] = _vpu_dot(
                q[u],
                lambda i, t: kt[g, r * 128 + i * 8:r * 128 + (i + 1) * 8, t * 128:(t + 1) * 128],
                score.get(g, [None] * NT))

        def probs(g):
            e, inv = _softmax(score[g], scale)
            prob[g] = [p.astype(BF16) for p in e], inv

        def weigh(h, lo, hi, step):
            for t in range(lo, hi, step):
                p = jnp.concatenate(prob[h // G][0][t:t + step], axis=1)
                if layer == 1:
                    words = pltpu.bitcast(vbuf[h, t * 128:(t + step) * 128, :], U32)
                    v_p[h, t * 64:(t + step) * 64, :] = words
                else:
                    words = v_p[h, t * 64:(t + step) * 64, :]
                r = _dot(p, words)
                out[h] = out[h] + r if h in out else r
            if hi == NT:
                r = out[h] * prob[h // G][1]
                out[h] = jnp.broadcast_to(r[h % G:h % G + 1, :], (G, DH))

        def values(h):
            weigh(h, 0, NT, 4)

        def last_values(n):
            head, lo, hi = LAST_PARTS[n]
            arrived(n)
            for h in range(head, head + 4):
                weigh(h, lo, hi, 1)

        def project_mxu(h):
            ob = out[h].astype(BF16)
            for n in range(ND):
                term = _dot(ob, wo_p[h, n])
                mxu_sum[n] = term if mxu_sum[n] is None else mxu_sum[n] + term

        def project_vpu(h):
            vpu_sum[:] = _vpu_dot(
                out[h], lambda i, n: wo_f[h, i * 8:(i + 1) * 8, n * 128:(n + 1) * 128],
                vpu_sum)

        if layer == 2:
            on_vpu = [*range(18), H - G]
            weighted = [(values, h, 64, {(probs, h // G): 200}) for h in range(H)]
            projected = [(project_mxu, h, 40, {(values, h): 120})
                         for h in range(H) if h not in on_vpu]
            mxu = [(query, u, 40, {}) for u in range(H - VPU_QUERIES)]
            mxu += weighted[:H - G] + projected[:1 - G] + weighted[H - G:] + projected[1 - G:]
            vpu = [(query_vpu, n, 8 * VPU_QUERIES, {}) for n in range(ND)]
            for u in range(H):
                needs = {(query, u): 300} if u < H - VPU_QUERIES else {}
                vpu.append((scores, u, 72, needs))
                if u and u % G == 0:
                    vpu.append((probs, u // G - 1, 16, {}))
            vpu.append((probs, NG - 1, 16, {}))
            vpu += [(project_vpu, h, 48, {(values, h): 220}) for h in on_vpu]
        elif arrived:
            mxu = [(values, h, 64, {}) for h in range(2 * G)] + [(arrived, None, 0, {})]
            mxu += [(values, h, 64, {}) for h in range(2 * G, 3 * G)]
            mxu += [(project_mxu, h, 40, {}) for h in range(2 * G, 3 * G)]
            for n, (head, _, hi) in enumerate(LAST_PARTS):
                mxu.append((last_values, n, 128, {(project_vpu, 2 * G - 1): 0}))
                if hi == NT:
                    mxu += [(project_mxu, h, 40, {}) for h in range(head, head + 4)]
            vpu = [(project_vpu, h, 40, {(values, h): 220}) for h in range(2 * G)]
        else:
            mxu = [(values, h, 64, {}) for h in range(H)]
            mxu += [(project_mxu, h, 40, {}) for h in range(H - 4, H)]
            vpu = [(project_vpu, h, 40, {(values, h): 220}) for h in range(H - 4)]
        _emit(mxu, vpu, extra)
        return residual(x, mxu_sum, vpu_sum)

    def stream(k_sem, v_sem):
        def start_cache(src, dst, sem, b, head, heads, row, queue):
            rows = 128 // heads
            if not isinstance(row, int):
                row = pl.multiple_of(row, rows)
            pltpu.make_async_copy(
                src.at[b, pl.ds(head, heads), pl.ds(SK - W + row, rows), :],
                dst.at[pl.ds(head, heads), pl.ds(row, rows), :], sem).start(priority=queue)

        def start_group(src, dst, sem, b, g, n, base=0):
            step, pair = divmod(n // 2, G // 2)
            start_cache(src, dst, sem, b, g * G + 2 * pair, 2,
                        (n % 2) * (W // 2) + step * 64 + base, n % 2)

        def start_keys(b, lo, hi):
            for n in range(lo, hi):
                start_group(k_hbm, kbuf, k_sem.at[n // NCOPY], b, n // NCOPY, n % NCOPY)

        def start_values(b, lo, hi):
            for n in range(lo, hi):
                start_group(v_hbm, vbuf, v_sem.at[n // (2 * NCOPY)], b, n // NCOPY, n % NCOPY)

        def wait(view, sem):
            pltpu.make_async_copy(view, view, sem).wait()

        def wait_keys(g):
            wait(kbuf.at[pl.ds(g * G, G)], k_sem.at[g])

        def start_weight(src, dst, sem, queue, row, rows, cols=slice(None)):
            index = (pl.ds(pl.multiple_of(row, rows), rows), cols)
            pltpu.make_async_copy(src.at[index], dst.at[index], sem).start(priority=queue)

        def start_wo(i):
            for part in range(8):
                start_weight(wo_hbm, wo_v, v_sem.at[1], part % 2, part * 512 + i * 16, 16)

        def start_mlp(i):
            for part in range(2):
                start_weight(w1t_hbm, w1t_v, v_sem.at[1], 0, part * (F // 2) + i * 16, 16)
                start_weight(w2_hbm, w2_v, v_sem.at[1], 1, part * (F // 2) + i * 16, 16)

        @pl.loop(0, 8)
        def _(i):
            for c in range(2):
                for part in range(10):
                    start_weight(wq_hbm, wq_v, v_sem.at[0], part % 2, part * 64 + i * 8, 8,
                                 pl.ds(c * 2048, 2048))

        small = [pltpu.make_async_copy(src, dst, k_sem.at[n])
                 for n, (src, dst) in enumerate(((x_hbm, x_v), (b1_hbm, b1_v), (b2_hbm, b2_v)))]
        for copy in small:
            copy.start()
        pl.loop(0, 6)(start_mlp)
        pl.loop(0, 8)(start_wo)
        for copy in small:
            copy.wait()
        wait(wq_v, v_sem.at[0])

        xs[...] = x_v[...].astype(F32)
        b2s[...] = jnp.broadcast_to(b2_v[...].astype(F32).reshape(1, D), (G, D))
        b1 = jnp.concatenate([b1_v[...].astype(F32).reshape(1, F),
                              jnp.zeros((1, NF * 128 - F), F32)], axis=1)
        for f in range(NF):
            b1s[f] = jnp.broadcast_to(b1[:, f * 128:(f + 1) * 128], (G, 128))
        ones = jnp.ones((G, D), BF16)
        mean, _, var = _moments(xs[...])
        y1 = ((xs[...] - mean) * lax.rsqrt(var + EPS)).astype(BF16)

        @pl.loop(0, 2 * NG)
        def _(step):
            g = step // 2

            @pl.when(step < NG)
            def _():
                for i in range(6):
                    start_wo(8 + step * 6 + i)

            @pl.when(step >= NG)
            def _():
                for i in range(12):
                    start_mlp(6 + (step - NG) * 12 + i)

            def reorder(lo, hi):
                for n in range(lo, hi):
                    columns = _interleave([
                        wq_v[n * 128:(n + 1) * 128, pl.ds(pl.multiple_of((g * G + j) * DH, DH), DH)]
                        for j in range(G)])
                    for u in range(G):
                        blk = jnp.concatenate(columns[u * 16:(u + 1) * 16], axis=0).T.astype(BF16)
                        wq_p[g * G + u, n * 64:(n + 1) * 64, :] = pltpu.bitcast(blk, U32)

            @pl.when(step % 2 == 0)
            def _():
                reorder(0, 3)

            @pl.when(step % 2 == 1)
            def _():
                for j in range(G):
                    head = pl.ds(pl.multiple_of((g * G + j) * DH, DH), DH)
                    q1[g * G + j] = jnp.dot(y1, wq_v[:, head], preferred_element_type=F32)
                reorder(3, ND)
                for u in range(G):
                    wq_sum[g * G + u] = _dot(ones, wq_p[g * G + u])

        start_keys(0, 0, NCOPY)
        for buf in (wo_v, w1t_v, w2_v):
            wait(buf, v_sem.at[1])
        for t in range(VPU_QUERIES):
            wq_f[:, t * 128:(t + 1) * 128] = (
                pltpu.bitcast(wq_p[H - VPU_QUERIES + t], BF16).astype(F32))

        def start_first_keys(i):
            for n in range(8):
                start_group(k_hbm, kbuf, k_sem.at[i // 8], 0, i // 8, n, (i % 8) * 64)

        @pl.loop(0, H // 2)
        def _(i):
            pl.when(i < 12)(lambda: start_first_keys(8 + i))
            for h in (2 * i, 2 * i + 1):
                head = pl.ds(pl.multiple_of(h * DH, DH), DH)
                blk = wo_v[head, :]
                wo_f[h] = blk.astype(F32)
                for n in range(ND):
                    wo_p[h, n] = pltpu.bitcast(blk[:, n * 128:(n + 1) * 128], U32)

        def arrange_mlp(f, up_t, down):
            up = jnp.concatenate([up_t[:, n * 128:(n + 1) * 128].T for n in range(ND)], axis=0)
            w1_p[f] = pltpu.bitcast(up, U32)
            w1_sum[f] = jnp.dot(ones, up, preferred_element_type=F32)
            w2_f[f] = down.astype(F32)
            for n in range(ND):
                w2_p[f, n] = pltpu.bitcast(down[:, n * 128:(n + 1) * 128], U32)

        @pl.loop(0, F // 128)
        def _(f):
            pl.when(f >= 1)(lambda: start_first_keys(19 + f))
            rows = pl.ds(pl.multiple_of(f * 128, 128), 128)
            arrange_mlp(f, w1t_v[rows, :], w2_v[rows, :])

        rows = pl.ds(F // 128 * 128, F % 128)
        pad = jnp.zeros((NF * 128 - F, D), BF16)
        arrange_mlp(NF - 1, jnp.concatenate([w1t_v[rows, :], pad], axis=0),
                    jnp.concatenate([w2_v[rows, :], pad], axis=0))
        for t in range(VPU_UP):
            w1_f[:, t * 128:(t + 1) * 128] = pltpu.bitcast(w1_p[NF - VPU_UP + t], BF16).astype(F32)
        wait_keys(0)
        wait_keys(1)

        @pl.loop(0, B)
        def _(b):
            start_values(b, 0, NCOPY)

            @pl.loop(0, NG)
            def _(g):
                pl.when(g >= 2)(lambda: wait_keys(g))
                keys_arrived(b, g)

                def more_values(*cuts):
                    for step in range(len(cuts) - 1):
                        pl.when(g == step)(functools.partial(start_values, b, *cuts[step:step + 2]))

                @pl.when(b < B - 1)
                def _():
                    more_values(64, 160, 256)
                    pl.when(g == 2)(lambda: start_keys(b + 1, 0, NCOPY))

                pl.when(b == B - 1)(lambda: more_values(64, 108, 152, 192))

            @pl.when(b < B - 1)
            def _():
                def burst(i):
                    fence()
                    start_keys(b + 1, KEY_BURSTS[i], KEY_BURSTS[i + 1])

                def bursts(*plan):
                    return [task for i, delay in plan
                            for task in ((lambda _: None, i, delay, {}), (burst, i, 0, {}))]

                burst(0)
                wait(vbuf.at[pl.ds(0, 2 * G)], v_sem.at[0])
                wait(vbuf.at[pl.ds(2 * G, 2 * G)], v_sem.at[1])
                x = jnp.broadcast_to(xs[pl.ds(b, 1), :], (G, D))
                x = attention(x, 1, bursts((1, 1300)))
                burst(2)
                x = mlp(x)
                burst(3)
                x = attention(x, 2, bursts((4, 1200), (5, 1250)))
                burst(6)
                xs[pl.ds(b, 1), :] = mlp(x)[:1]
                burst(7)
                wait_keys(0)
                wait_keys(1)

        for head in (H - 8, H - 4):
            for row in range(0, W // 2, 32):
                for queue in range(2):
                    tile = (queue * (W // 2) + row) // 128
                    n, = [n for n, (h, lo, hi) in enumerate(LAST_PARTS)
                          if h == head and lo <= tile < hi]
                    start_cache(v_hbm, vbuf, k_sem.at[n], B - 1, head, 4,
                                queue * (W // 2) + row, queue)
        wait(vbuf.at[pl.ds(0, 2 * G)], v_sem.at[0])

        def arrived(n):
            if n is None:
                wait(vbuf.at[pl.ds(2 * G, G)], v_sem.at[1])
            else:
                head, lo, hi = LAST_PARTS[n]
                wait(vbuf.at[pl.ds(head, 4), pl.ds(lo * 128, (hi - lo) * 128)], k_sem.at[n])

        x = jnp.broadcast_to(xs[B - 1:, :], (G, D))
        return attention(x, 1, arrived=arrived)

    x = pl.run_scoped(stream, pltpu.SemaphoreType.DMA((NG,)), pltpu.SemaphoreType.DMA((2,)))
    fence()
    x = attention(mlp(x), 2)
    fence()
    x = mlp(x, vpu_down=5)
    last = lax.broadcasted_iota(jnp.int32, (B, D), 0) == B - 1
    o_ref[...] = jnp.where(last, x, xs[...]).astype(o_ref.dtype)


@jax.jit
def pallas_interleave_layers__sliding_block_cached__mixer_channel_mlp__decode_kernel(
    A_x: jax.Array,
    A_k_cache: jax.Array,
    A_v_cache: jax.Array,
    A_wq: jax.Array,
    A_wo: jax.Array,
    B_x: jax.Array,
    B_w1: jax.Array,
    B_b1: jax.Array,
    B_w2: jax.Array,
    B_b2: jax.Array,
):
    del B_x
    out = pl.pallas_call(
        _kernel,
        out_shape=jax.ShapeDtypeStruct((B, D), A_x.dtype),
        in_specs=[pl.BlockSpec(memory_space=pl.ANY)] * 9,
        out_specs=pl.BlockSpec(memory_space=pltpu.VMEM),
        scratch_shapes=[
            pltpu.VMEM((NG, DH * G, W), F32),
            pltpu.VMEM((H, W // 2, DH), U32),
            pltpu.VMEM((H, D // 2, 128), U32),
            pltpu.VMEM((H, ND, DH // 2, 128), U32),
            pltpu.VMEM((NF, D // 2, 128), U32),
            pltpu.VMEM((NF, ND, 64, 128), U32),
            pltpu.VMEM((D, VPU_QUERIES * 128), F32),
            pltpu.VMEM((H, DH, D), F32),
            pltpu.VMEM((D, VPU_UP * 128), F32),
            pltpu.VMEM((NF, 128, D), F32),
            pltpu.VMEM((H, G, 128), F32),
            pltpu.VMEM((NF, G, 128), F32),
            pltpu.VMEM((NF, G, 128), F32),
            pltpu.VMEM((G, D), F32),
            pltpu.VMEM((B, D), F32),
            pltpu.VMEM((H, B, DH), F32),
            pltpu.VMEM((NG, G, W), F32),
            pltpu.VMEM((NG, G, 128), F32),
            pltpu.VMEM((H, W, DH), BF16),
            pltpu.VMEM((H, W, DH), BF16),
            pltpu.VMEM((D, H * DH), BF16),
            pltpu.VMEM((H * DH, D), BF16),
            pltpu.VMEM((F, D), BF16),
            pltpu.VMEM((F, D), BF16),
            pltpu.VMEM((B, D), BF16),
            pltpu.VMEM((F,), BF16),
            pltpu.VMEM((D,), BF16),
            pltpu.SemaphoreType.REGULAR,
        ],
        compiler_params=pltpu.CompilerParams(
            vmem_limit_bytes=110 * 1024 * 1024,
            disable_bounds_checks=True),
    )(A_x.reshape(B, D), A_k_cache, A_v_cache, A_wq, A_wo, B_w1.T, B_b1, B_w2, B_b2)
    return out.reshape(B, 1, D)
```
